```python
import jax
import jax.numpy as jnp

def _softmax(x, axis=-1):
    return jax.nn.softmax(x, axis=axis)
def _gelu(x):
    return jax.nn.gelu(x, approximate=True)
def _silu(x):
    return jax.nn.silu(x)
def _sigmoid(x):
    return jax.nn.sigmoid(x)
def _layernorm(x, axis=-1, eps=1e-5):
    m = jnp.mean(x, axis=axis, keepdims=True)
    v = jnp.var(x, axis=axis, keepdims=True)
    return (x - m) / jnp.sqrt(v + eps)
def _scatter_add(tgt, idx, src, axis=0):
    return tgt.at[idx].add(src)
def _segment_sum(src, seg, n):
    return jax.ops.segment_sum(src, seg, n)
class _Rng:
    def __init__(self, key):
        self._k = key
    def _next(self):
        self._k, sub = jax.random.split(self._k)
        return sub
    def normal(self, shape):
        return jax.random.normal(self._next(), shape, dtype=jnp.bfloat16)
    def randint(self, lo, hi, shape):
        return jax.random.randint(self._next(), shape, lo, hi, dtype=jnp.int32)
    def uniform(self, shape, lo=0.0, hi=1.0):
        return jax.random.uniform(self._next(), shape, jnp.bfloat16, lo, hi)
    def permutation(self, n):
        return jax.random.permutation(self._next(), n)


kernel_name = 'standalone__modern_conv_block_slak__vision'

def setup_inputs():
    _rng = _Rng(jax.random.key(int.from_bytes(__import__("os").urandom(4), "little")))
    _w = (lambda a: (lambda t: t.astype(jnp.bfloat16) if jnp.issubdtype(t.dtype, jnp.floating) else t)(jnp.asarray(a)))
    H = W = 384
    C = 384
    K = 1
    return {
        "x": _w((lambda *s: _rng.normal(s) * 0.05)(1, H, W, C)),
        "dw": _w((lambda *s: _rng.normal(s) * 0.05)(K, K, C)),
        "w1": _w((lambda *s: _rng.normal(s) * 0.05)(C, 4 * C)),
        "w2": _w((lambda *s: _rng.normal(s) * 0.05)(4 * C, C)),
        "grn_g": _w((lambda *s: _rng.normal(s) * 0.05)(4 * C)),
        "grn_b": _w((lambda *s: _rng.normal(s) * 0.05)(4 * C)),
    }

def reference(x, dw, w1, w2, grn_g, grn_b):
    B, H, W, C = x.shape
    K = dw.shape[0]
    pad = K // 2
    xp = jnp.pad(x, ((0,0),(pad,pad),(pad,pad),(0,0)))
    out = jnp.zeros_like(x)
    for i in range(K):
        for j in range(K):
            out = out + xp[:, i:i+H, j:j+W, :] * dw[i, j][None, None, None, :]
    h = _layernorm(out, axis=-1)
    h = _gelu(h @ w1)
    gx = jnp.sqrt((h * h).sum(axis=(1, 2), keepdims=True) + 1e-6)
    nx = gx / (gx.mean(axis=-1, keepdims=True) + 1e-6)
    h = grn_g[None, None, None, :] * (h * nx) + grn_b[None, None, None, :] + h
    return x + h @ w2
```

```python
import functools
import math

import jax
import jax.numpy as jnp
import jax.experimental.pallas as pl
import jax.experimental.pallas.tpu as pltpu

_LN_EPS = 1e-5
_GRN_EPS = 1e-6
_C0 = math.sqrt(2.0 / math.pi)
_C1 = 0.044715 * _C0
_BETA = _C1 ** (1.0 / 3.0)
_KAPPA = _C0 / _BETA
_HSCALE = 1.0 / (2.0 * _BETA)


def _kernel(x_hbm, dw_ref, w1_ref, w2_ref, g_ref, b_ref, o_hbm, h_hbm,
            xbuf, obuf, hbuf, w2s, acc, xn_a, xn_b, xsem, osem, hsem, *, cfg):
    TM, T, G, NCACHE, NS, NX, NO = (cfg[k] for k in ("TM", "T", "G", "NCACHE", "NS", "NX", "NO"))
    SM1, NC1, SM2 = cfg["SM1"], cfg["NC1"], cfg["SM2"]
    C, F = w1_ref.shape
    xn_bufs = (xn_a, xn_b)

    def cached(i):
        return jnp.logical_and(i % G == G - 1, i // G < NCACHE)

    def sidx(i):
        return i - jnp.minimum(i // G, NCACHE)

    def slot_of(i):
        return jnp.where(cached(i), NS + i // G, sidx(i) % NS)

    def x_copy(i, k):
        return pltpu.make_async_copy(x_hbm.at[pl.ds(i * TM, TM)], xbuf.at[k % NX], xsem.at[k % NX])

    def o_copy(i):
        return pltpu.make_async_copy(obuf.at[i % NO], o_hbm.at[pl.ds(i * TM, TM)], osem.at[i % NO])

    def h_store(s):
        return pltpu.make_async_copy(hbuf.at[s % NS], h_hbm.at[pl.ds(s * TM, TM)], hsem.at[s % NS])

    def h_load(s):
        return pltpu.make_async_copy(h_hbm.at[pl.ds(s * TM, TM)], hbuf.at[s % NS], hsem.at[s % NS])

    NSTREAM = T - NCACHE
    for k in range(NX - 1):
        x_copy(k, k).start()
    acc[...] = jnp.zeros_like(acc)
    dw = dw_ref[...].astype(jnp.float32)

    def layernorm(xs, r0, n, dst):
        y = xbuf[xs, r0:r0 + n, :].astype(jnp.float32) * dw
        m = jnp.sum(y, axis=-1, keepdims=True) * (1.0 / C)
        d = y - m
        v = jnp.sum(d * d, axis=-1, keepdims=True) * (1.0 / C)
        xn = (d * (jax.lax.rsqrt(v + _LN_EPS) * _BETA)).astype(jnp.bfloat16)
        q0 = (r0 % SM1) // 2
        dst[q0:q0 + n // 2, :] = pltpu.bitcast(xn, jnp.uint32)

    x_copy(0, 0).wait()
    layernorm(0, 0, SM1, xn_bufs[0])
    S = TM // SM1
    assert S % 2 == 0
    NCH = F // NC1
    LNP = cfg.get("LNP", NCH)

    def phase1(i, carry):
        nxt = i + NX - 1
        x_copy(jnp.where(nxt < T, nxt, nxt - T), nxt).start()
        s = sidx(i)
        is_stream = jnp.logical_not(cached(i))

        @pl.when(jnp.logical_and(is_stream, s >= NS))
        def _():
            h_store(s - NS).wait()

        x_copy(jnp.where(i + 1 < T, i + 1, 0), i + 1).wait()
        slot = slot_of(i)

        for r in range(S):
            src, dst = xn_bufs[r % 2], xn_bufs[(r + 1) % 2]
            xs_n = (i % NX) if r + 1 < S else ((i + 1) % NX)
            r_n = ((r + 1) % S) * SM1
            rows = slice(r * SM1, (r + 1) * SM1)
            xn = pltpu.bitcast(src[...], jnp.bfloat16)
            for j in range(NCH):
                cols = slice(j * NC1, (j + 1) * NC1)
                if cfg.get("LNPOS", 0) == 0:
                    for p in range(j * LNP // NCH, (j + 1) * LNP // NCH):
                        layernorm(xs_n, r_n + p * (SM1 // LNP), SM1 // LNP, dst)
                w = jnp.dot(xn, w1_ref[:, cols], preferred_element_type=jnp.float32)
                t = jnp.tanh(w * (w * w + _KAPPA))
                h = w * t + w
                hbuf[slot, rows, cols] = h.astype(jnp.bfloat16)
                acc[:, cols] += jnp.sum((h * h).reshape(SM1 // 8, 8, NC1), axis=0)
                if cfg.get("LNPOS", 0) == 1:
                    for p in range(j * LNP // NCH, (j + 1) * LNP // NCH):
                        layernorm(xs_n, r_n + p * (SM1 // LNP), SM1 // LNP, dst)

        @pl.when(is_stream)
        def _():
            h_store(s).start()

        return carry

    jax.lax.fori_loop(0, T, phase1, 0)

    for s in range(NSTREAM - NS, NSTREAM):
        h_store(s).wait()
    for s in range(NS - 1):
        h_load(s).start()

    gx = jnp.sqrt(jnp.sum(acc[...], axis=0, keepdims=True) * (_HSCALE * _HSCALE) + _GRN_EPS)
    nx = gx / (jnp.sum(gx, axis=-1, keepdims=True) * (1.0 / F) + _GRN_EPS)
    sc = (g_ref[...].astype(jnp.float32) * nx + 1.0) * _HSCALE
    for k in range(F // 128):
        ks = slice(k * 128, (k + 1) * 128)
        col = jnp.transpose(jnp.broadcast_to(sc[:, ks], (128, 128)))
        for n in range(C // 128):
            ns = slice(n * 128, (n + 1) * 128)
            w2s[ks, ns] = (w2_ref[ks, ns].astype(jnp.float32) * col).astype(jnp.bfloat16)
    bias = jnp.dot(jnp.broadcast_to(b_ref[...], (16, F)), w2_ref[...],
                   preferred_element_type=jnp.float32)[0:1, :]

    def phase2(i, carry):
        k = T + i
        nxt = i + NX - 1

        @pl.when(nxt < T)
        def _():
            x_copy(nxt, T + nxt).start()

        s = sidx(i)
        is_stream = jnp.logical_not(cached(i))

        @pl.when(is_stream)
        def _():
            @pl.when(s + NS - 1 < NSTREAM)
            def _():
                h_load(s + NS - 1).start()
            h_load(s).wait()

        @pl.when(i >= NO)
        def _():
            o_copy(i - NO).wait()

        @pl.when(i > 0)
        def _():
            x_copy(i, k).wait()
        slot = slot_of(i)
        xs = k % NX
        os_ = i % NO

        def sub(r, c):
            rows = pl.ds(r * SM2, SM2)
            y = jnp.dot(hbuf[slot, rows, :], w2s[...], preferred_element_type=jnp.float32)
            obuf[os_, rows, :] = (y + bias + xbuf[xs, rows, :].astype(jnp.float32)).astype(obuf.dtype)
            return c

        for r in range(TM // SM2):
            sub(r, 0)
        o_copy(i).start()
        return carry

    jax.lax.fori_loop(0, T, phase2, 0)
    for i in range(T - NO, T):
        o_copy(i).wait()


_DEFAULT_CFG = dict(TM=2048, G=5, NCACHE=13, NS=3, NX=3, NO=2, SM1=128, NC1=512, SM2=256, LNP=1, VMEM_MB=124)


def _run(x, dw, w1, w2, grn_g, grn_b, cfg):
    B, H, W, C = x.shape
    F = w1.shape[1]
    assert B == 1 and dw.shape[:2] == (1, 1)
    N = B * H * W
    cfg = dict(cfg)
    TM = cfg["TM"]
    assert N % TM == 0
    cfg["T"] = N // TM
    out, _ = pl.pallas_call(
        functools.partial(_kernel, cfg=cfg),
        in_specs=[pl.BlockSpec(memory_space=pl.ANY)] + [pl.BlockSpec(memory_space=pltpu.VMEM)] * 5,
        out_specs=[pl.BlockSpec(memory_space=pl.ANY)] * 2,
        out_shape=[
            jax.ShapeDtypeStruct((N, C), x.dtype),
            jax.ShapeDtypeStruct(((cfg["T"] - cfg["NCACHE"]) * TM, F), jnp.bfloat16),
        ],
        scratch_shapes=[
            pltpu.VMEM((cfg["NX"], TM, C), x.dtype),
            pltpu.VMEM((cfg["NO"], TM, C), x.dtype),
            pltpu.VMEM((cfg["NS"] + cfg["NCACHE"], TM, F), jnp.bfloat16),
            pltpu.VMEM((F, C), jnp.bfloat16),
            pltpu.VMEM((8, F), jnp.float32),
            pltpu.VMEM((cfg['SM1'] // 2, C), jnp.uint32),
            pltpu.VMEM((cfg['SM1'] // 2, C), jnp.uint32),
            pltpu.SemaphoreType.DMA((cfg["NX"],)),
            pltpu.SemaphoreType.DMA((cfg["NO"],)),
            pltpu.SemaphoreType.DMA((cfg["NS"],)),
        ],
        compiler_params=pltpu.CompilerParams(vmem_limit_bytes=cfg["VMEM_MB"] * 1024 * 1024),
    )(
        x.reshape(N, C),
        dw.reshape(1, C),
        w1.astype(jnp.bfloat16),
        w2.astype(jnp.bfloat16),
        grn_g.reshape(1, F),
        grn_b.reshape(1, F).astype(jnp.bfloat16),
    )
    return out.reshape(B, H, W, C)


@jax.jit
def pallas_standalone__modern_conv_block_slak__vision_kernel(
    x: jax.Array,
    dw: jax.Array,
    w1: jax.Array,
    w2: jax.Array,
    grn_g: jax.Array,
    grn_b: jax.Array,
):
    return _run(x, dw, w1, w2, grn_g, grn_b, _DEFAULT_CFG)
```

```python
import functools
import math

import jax
import jax.numpy as jnp
import jax.experimental.pallas as pl
import jax.experimental.pallas.tpu as pltpu

_LN_EPS = 1e-5
_GRN_EPS = 1e-6
_C0 = math.sqrt(2.0 / math.pi)
_BETA = (0.044715 * _C0) ** (1.0 / 3.0)
_KAPPA = _C0 / _BETA
_HSCALE = 1.0 / (2.0 * _BETA)

_W_COMBOS = {
    1: {(0, 0): 1, (0, 2): -1, (1, 0): -1},
    2: {(0, 0): 1, (0, 1): -1, (2, 0): -1},
    3: {(1, 1): 1, (0, 1): -1, (1, 2): -1},
    4: {(1, 1): 1, (1, 0): -1, (2, 1): -1},
    5: {(2, 2): 1, (0, 2): -1, (2, 1): -1},
    6: {(1, 2): 1, (2, 0): 1, (2, 2): -1},
    7: {(0, 1): 1},
    8: {(1, 0): 1, (0, 1): -1},
    9: {(1, 0): -1},
    10: {(2, 1): 1},
    11: {(1, 2): 1, (2, 1): -1},
    12: {(1, 2): -1},
    13: {(2, 0): 1, (0, 2): -1},
    14: {(2, 0): 1},
    15: {(0, 2): 1},
}
_SHARED = {"q8": ("m7", "m8"), "q9": ("q8", "m9"), "q11": ("m10", "m11"), "q12": ("q11", "m12")}
_OUTPUTS = {
    (0, 0): {"m1": 1, "m2": 1, "q8": 1, "m13": 1, "m15": 1},
    (0, 1): {"m3": 1, "m7": 1, "q12": 1},
    (0, 2): {"m5": 1, "q12": 1, "m15": 1},
    (1, 0): {"m2": 1, "q9": 1, "m14": 1},
    (1, 1): {"m4": 1, "q9": 1, "m10": 1},
    (1, 2): {"m5": 1, "m6": 1, "q11": 1, "m13": -1, "m14": 1},
}


def _a_combos(a):
    (a11, a21, a31), (a12, a22, a32) = a
    c1, c6 = a11 - a12, a31 - a32
    c8, c11 = c1 + a21, a22 - c6
    return {1: c1, 6: c6, 7: a11 + a21, 8: c8, 9: c8 - a22, 10: a22 + a32, 11: c11, 12: c11 - a21,
            13: a12 + a31, 14: a12 + a32, 15: a11 + a31}


_A_SINGLE = {2: (1, 0), 3: (0, 1), 4: (1, 1), 5: (0, 2)}


def _w_combo(r, block):
    pos = [block(*pq) for pq, sign in _W_COMBOS[r].items() if sign > 0]
    neg = [block(*pq) for pq, sign in _W_COMBOS[r].items() if sign < 0]
    total = functools.reduce(lambda u, v: u + v, pos) if pos else -neg.pop()
    return functools.reduce(lambda u, v: u - v, neg, total)


def _block_product(order, product, emit):
    ready, partial = {}, {}
    missing = {iq: dict(terms) for iq, terms in _OUTPUTS.items()}
    for r in order:
        fresh = ["m%d" % r]
        ready[fresh[0]] = product(r)
        for name, (u, v) in _SHARED.items():
            if name not in ready and u in ready and v in ready:
                ready[name] = ready[u] + ready[v]
                fresh.append(name)
        for iq, terms in missing.items():
            for name in fresh:
                if name not in terms:
                    continue
                sign = terms.pop(name)
                if iq not in partial:
                    partial[iq] = (sign, ready[name])
                else:
                    have, value = partial[iq]
                    if have == sign:
                        partial[iq] = (have, value + ready[name])
                    elif have > 0:
                        partial[iq] = (1, value - ready[name])
                    else:
                        partial[iq] = (1, ready[name] - value)
                if not terms:
                    emit(*iq, partial[iq][1])


def _pack(v):
    return pltpu.bitcast(v.astype(jnp.bfloat16), jnp.uint32)


def _unpack(v):
    return pltpu.bitcast(v, jnp.bfloat16)


def _kernel(x_hbm, dw_ref, w1_ref, w2_ref, g_ref, b_ref, o_hbm, h_hbm,
            xbuf, obuf, hbuf, wc1, wc2, lhs0, acc, xsem, osem, hsem, *, cfg):
    TM, T, G, NCACHE, NS, NX, NO = (cfg[k] for k in ("TM", "T", "G", "NCACHE", "NS", "NX", "NO"))
    R1, R2 = cfg["R1"], cfg["R2"]
    C, F = w1_ref.shape
    CB, FB = C // 3, F // 3
    NSTREAM = T - NCACHE
    f32, bf16 = jnp.float32, jnp.bfloat16

    def cached(t):
        return jnp.logical_and(t % G == 0, t // G < NCACHE)

    def stream_index(t):
        return t - jnp.minimum((t + G - 1) // G, NCACHE)

    def slot_of(t):
        return jnp.where(cached(t), NS + t // G, stream_index(t) % NS)

    def tile_of(step):
        return jnp.where(step < T, step, 2 * T - 1 - step)

    def x_copy(step):
        rows = pl.ds(tile_of(step) * TM, TM)
        return pltpu.make_async_copy(x_hbm.at[rows], xbuf.at[step % NX], xsem.at[step % NX])

    def o_copy(step):
        rows = pl.ds(tile_of(step) * TM, TM)
        return pltpu.make_async_copy(obuf.at[step % NO], o_hbm.at[rows], osem.at[step % NO])

    def h_store(s):
        rows = pl.ds(s * (TM // 2), TM // 2)
        return pltpu.make_async_copy(hbuf.at[s % NS], h_hbm.at[rows], hsem.at[s % NS])

    def h_load(s):
        rows = pl.ds(s * (TM // 2), TM // 2)
        return pltpu.make_async_copy(h_hbm.at[rows], hbuf.at[s % NS], hsem.at[s % NS])

    for step in range(NX - 1):
        x_copy(step).start()

    for r in _W_COMBOS:
        wc1[r - 1] = _pack(_w_combo(
            r, lambda p, q: w1_ref[p * CB:(p + 1) * CB, q * FB:(q + 1) * FB].astype(f32)))
    acc[...] = jnp.zeros_like(acc)
    dw = dw_ref[...].astype(f32)

    def layernorm(xs, r0):
        y = xbuf[xs, r0:r0 + R1, :].astype(f32) * dw
        d = y - jnp.sum(y, axis=-1, keepdims=True) * (1.0 / C)
        v = jnp.sum(d * d, axis=-1, keepdims=True)
        return d * jax.lax.rsqrt(v * (1.0 / (C * _BETA ** 2)) + _LN_EPS / _BETA ** 2)

    def lhs1(xs, r0):
        rows = [layernorm(xs, r0 + i * R1) for i in range(2)]
        a = [[u[:, p * CB:(p + 1) * CB] for p in range(3)] for u in rows]
        ops = _a_combos(a)
        ops.update({r: a[i][p] for r, (i, p) in _A_SINGLE.items()})
        return {r: v.astype(bf16) for r, v in ops.items()}

    x_copy(0).wait()
    for r, v in lhs1(0, 0).items():
        lhs0[r - 1] = pltpu.bitcast(v, jnp.uint32)

    def sweep1(t, carry):
        x_copy(t + NX - 1).start()
        s = stream_index(t)
        streamed = jnp.logical_not(cached(t))

        @pl.when(jnp.logical_and(streamed, s >= NS))
        def _():
            h_store(s - NS).wait()

        x_copy(t + 1).wait()
        slot = slot_of(t)
        nsub = TM // (2 * R1)
        sumsq = [None] * 3
        lhs = {r: _unpack(lhs0[r - 1]) for r in _W_COMBOS}
        for sub in range(nsub):
            r0 = sub * 2 * R1
            nxt = lhs1(t % NX, r0 + 2 * R1) if sub + 1 < nsub else lhs1((t + 1) % NX, 0)

            def product(r):
                return jnp.dot(lhs[r], _unpack(wc1[r - 1]), preferred_element_type=f32)

            def emit(i, q, w):
                h = w * jnp.tanh(w * (w * w + _KAPPA)) + w
                row = (r0 + i * R1) // 2
                hbuf[slot, row:row + R1 // 2, q * FB:(q + 1) * FB] = _pack(h)
                sq = jnp.sum((h * h).reshape(R1 // 8, 8, FB), axis=0)
                sumsq[q] = sq if sumsq[q] is None else sumsq[q] + sq

            _block_product(cfg["ORDER1"], product, emit)
            lhs = nxt
        for q in range(3):
            acc[:, q * FB:(q + 1) * FB] += sumsq[q]
        for r, v in lhs.items():
            lhs0[r - 1] = pltpu.bitcast(v, jnp.uint32)

        @pl.when(jnp.logical_and(streamed, s < NSTREAM - NS))
        def _():
            h_store(s).start()

        return carry

    jax.lax.fori_loop(0, T, sweep1, 0)

    gx = jnp.sqrt(jnp.sum(acc[...], axis=0, keepdims=True) * _HSCALE ** 2 + _GRN_EPS)
    nx = gx / (jnp.sum(gx, axis=-1, keepdims=True) * (1.0 / F) + _GRN_EPS)
    scale = (g_ref[...].astype(f32) * nx + 1.0) * _HSCALE
    for k in range(FB // CB):
        col = [jnp.transpose(jnp.broadcast_to(scale[:, p * FB + k * CB:p * FB + (k + 1) * CB], (CB, CB)))
               for p in range(3)]
        scaled = [[w2_ref[p * FB + k * CB:p * FB + (k + 1) * CB, q * CB:(q + 1) * CB].astype(f32) * col[p]
                   for q in range(3)] for p in range(3)]
        for r in _W_COMBOS:
            wc2[r - 1, k * CB // 2:(k + 1) * CB // 2, :] = _pack(_w_combo(r, lambda p, q: scaled[p][q]))
    bias = jnp.dot(jnp.broadcast_to(b_ref[...], (16, F)), w2_ref[...], preferred_element_type=f32)[0:1, :]

    def sweep2(step, carry):
        t = 2 * T - 1 - step

        @pl.when(step + NX - 1 < 2 * T)
        def _():
            x_copy(step + NX - 1).start()

        s = stream_index(t)
        streamed = jnp.logical_not(cached(t))

        @pl.when(jnp.logical_and(streamed, s < NSTREAM - NS))
        def _():
            h_load(s).wait()

        @pl.when(step >= T + NO)
        def _():
            o_copy(step - NO).wait()

        @pl.when(step > T)
        def _():
            x_copy(step).wait()

        slot = slot_of(t)
        xs = step % NX
        os_ = step % NO
        for sub in range(TM // (2 * R2)):
            r0 = sub * 2 * R2

            def block(i, p):
                row = (r0 + i * R2) // 2
                return _unpack(hbuf[slot, row:row + R2 // 2, p * FB:(p + 1) * FB])

            ops = _a_combos([[block(i, p).astype(f32) for p in range(3)] for i in range(2)])

            def product(r):
                lhs = block(*_A_SINGLE[r]) if r in _A_SINGLE else ops[r].astype(bf16)
                return jnp.dot(lhs, _unpack(wc2[r - 1]), preferred_element_type=f32)

            def emit(i, q, y):
                rows, cols = slice(r0 + i * R2, r0 + (i + 1) * R2), slice(q * CB, (q + 1) * CB)
                obuf[os_, rows, cols] = (y + bias[:, cols] + xbuf[xs, rows, cols].astype(f32)).astype(obuf.dtype)

            _block_product(cfg["ORDER2"], product, emit)

        o_copy(step).start()

        @pl.when(jnp.logical_and(streamed, s >= NS))
        def _():
            h_load(s - NS).start()

        return carry

    jax.lax.fori_loop(T, 2 * T, sweep2, 0)
    for step in range(2 * T - NO, 2 * T):
        o_copy(step).wait()


_DEFAULT_CFG = dict(
    TM=2048, G=4, NCACHE=15, NS=3, NX=3, NO=2, R1=32, R2=32, VMEM_MB=127,
    ORDER1=(7, 8, 9, 2, 14, 10, 4, 11, 12, 3, 15, 5, 13, 1, 6),
    ORDER2=(7, 8, 9, 10, 4, 11, 12, 3, 15, 5, 2, 14, 13, 1, 6),
)


def _run(x, dw, w1, w2, grn_g, grn_b, cfg):
    B, H, W, C = x.shape
    F = w1.shape[1]
    assert B == 1 and dw.shape[:2] == (1, 1)
    N = H * W
    TM = cfg["TM"]
    assert N % TM == 0
    T = N // TM
    cfg = dict(cfg, T=T)
    assert (cfg["NCACHE"] - 1) * cfg["G"] < T
    n_spilled = T - cfg["NCACHE"] - cfg["NS"]
    out, _ = pl.pallas_call(
        functools.partial(_kernel, cfg=cfg),
        in_specs=[pl.BlockSpec(memory_space=pl.ANY)] + [pl.BlockSpec(memory_space=pltpu.VMEM)] * 5,
        out_specs=[pl.BlockSpec(memory_space=pl.ANY)] * 2,
        out_shape=[
            jax.ShapeDtypeStruct((N, C), x.dtype),
            jax.ShapeDtypeStruct((n_spilled * TM // 2, F), jnp.uint32),
        ],
        scratch_shapes=[
            pltpu.VMEM((cfg["NX"], TM, C), x.dtype),
            pltpu.VMEM((cfg["NO"], TM, C), x.dtype),
            pltpu.VMEM((cfg["NS"] + cfg["NCACHE"], TM // 2, F), jnp.uint32),
            pltpu.VMEM((15, C // 6, F // 3), jnp.uint32),
            pltpu.VMEM((15, F // 6, C // 3), jnp.uint32),
            pltpu.VMEM((15, cfg["R1"] // 2, C // 3), jnp.uint32),
            pltpu.VMEM((8, F), jnp.float32),
            pltpu.SemaphoreType.DMA((cfg["NX"],)),
            pltpu.SemaphoreType.DMA((cfg["NO"],)),
            pltpu.SemaphoreType.DMA((cfg["NS"],)),
        ],
        compiler_params=pltpu.CompilerParams(
            vmem_limit_bytes=int(cfg["VMEM_MB"] * 1024 * 1024), flags=cfg.get("FLAGS")),
    )(
        x.reshape(N, C),
        dw.reshape(1, C),
        w1.astype(jnp.bfloat16),
        w2.astype(jnp.bfloat16),
        grn_g.reshape(1, F),
        grn_b.reshape(1, F).astype(jnp.bfloat16),
    )
    return out.reshape(B, H, W, C)


@jax.jit
def pallas_standalone__modern_conv_block_slak__vision_kernel(
    x: jax.Array,
    dw: jax.Array,
    w1: jax.Array,
    w2: jax.Array,
    grn_g: jax.Array,
    grn_b: jax.Array,
):
    return _run(x, dw, w1, w2, grn_g, grn_b, _DEFAULT_CFG)
```

```python
import functools
import math

import jax
import jax.numpy as jnp
import jax.experimental.pallas as pl
import jax.experimental.pallas.tpu as pltpu

_LN_EPS = 1e-5
_GRN_EPS = 1e-6
_C0 = math.sqrt(2.0 / math.pi)
_BETA = (0.044715 * _C0) ** (1.0 / 3.0)
_KAPPA = _C0 / _BETA
_HSCALE = 1.0 / (2.0 * _BETA)

_HK = dict(
    sums={"s1": ("a00", -1, "a10"), "s6": ("a02", -1, "a12"), "s7": ("a00", 1, "a01"), "s8": ("s1", 1, "a01"),
          "s9": ("s8", -1, "a11"), "s10": ("a11", 1, "a12"), "s11": ("a11", -1, "s6"), "s12": ("s11", -1, "a01"),
          "s13": ("a10", 1, "a02"), "s14": ("a10", 1, "a12"), "s15": ("a00", 1, "a02")},
    left={1: "s1", 2: "a10", 3: "a01", 4: "a11", 5: "a02", 6: "s6", 7: "s7", 8: "s8", 9: "s9", 10: "s10",
          11: "s11", 12: "s12", 13: "s13", 14: "s14", 15: "s15"},
    right={
        1: {(0, 0): 1, (0, 2): -1, (1, 0): -1},
        2: {(0, 0): 1, (0, 1): -1, (2, 0): -1},
        3: {(1, 1): 1, (0, 1): -1, (1, 2): -1},
        4: {(1, 1): 1, (1, 0): -1, (2, 1): -1},
        5: {(2, 2): 1, (0, 2): -1, (2, 1): -1},
        6: {(1, 2): 1, (2, 0): 1, (2, 2): -1},
        7: {(0, 1): 1},
        8: {(1, 0): 1, (0, 1): -1},
        9: {(1, 0): -1},
        10: {(2, 1): 1},
        11: {(1, 2): 1, (2, 1): -1},
        12: {(1, 2): -1},
        13: {(2, 0): 1, (0, 2): -1},
        14: {(2, 0): 1},
        15: {(0, 2): 1},
    },
    shared={"q8": ("m7", "m8"), "q9": ("q8", "m9"), "q11": ("m10", "m11"), "q12": ("q11", "m12")},
    outputs={
        (0, 0): {"m1": 1, "m2": 1, "q8": 1, "m13": 1, "m15": 1},
        (0, 1): {"m3": 1, "m7": 1, "q12": 1},
        (0, 2): {"m5": 1, "q12": 1, "m15": 1},
        (1, 0): {"m2": 1, "q9": 1, "m14": 1},
        (1, 1): {"m4": 1, "q9": 1, "m10": 1},
        (1, 2): {"m5": 1, "m6": 1, "q11": 1, "m13": -1, "m14": 1},
    },
)


def _left_operands(scheme, a):
    vals = {"a%d%d" % (i, p): a[i][p] for i in range(2) for p in range(3)}
    for name, (u, sign, v) in scheme["sums"].items():
        vals[name] = vals[u] + vals[v] if sign > 0 else vals[u] - vals[v]
    return {r: vals[name] for r, name in scheme["left"].items()}


def _right_operand(scheme, r, block):
    pos = [block(*pq) for pq, sign in scheme["right"][r].items() if sign > 0]
    neg = [block(*pq) for pq, sign in scheme["right"][r].items() if sign < 0]
    total = functools.reduce(lambda u, v: u + v, pos) if pos else -neg.pop()
    return functools.reduce(lambda u, v: u - v, neg, total)


class _BlockProduct:
    def __init__(self, scheme, product, emit):
        self.scheme, self.product, self.emit = scheme, product, emit
        self.ready, self.partial = {}, {}
        self.missing = {iq: dict(terms) for iq, terms in scheme["outputs"].items()}

    def step(self, r):
        ready, partial = self.ready, self.partial
        fresh = ["m%d" % r]
        ready[fresh[0]] = self.product(r)
        for name, (u, v) in self.scheme["shared"].items():
            if name not in ready and u in ready and v in ready:
                ready[name] = ready[u] + ready[v]
                fresh.append(name)
        for iq, terms in self.missing.items():
            for name in fresh:
                if name not in terms:
                    continue
                sign = terms.pop(name)
                if iq not in partial:
                    partial[iq] = (sign, ready[name])
                else:
                    have, value = partial[iq]
                    if have == sign:
                        partial[iq] = (have, value + ready[name])
                    elif have > 0:
                        partial[iq] = (1, value - ready[name])
                    else:
                        partial[iq] = (1, ready[name] - value)
                if not terms:
                    self.emit(*iq, partial[iq][1])


def _pack(v):
    return pltpu.bitcast(v.astype(jnp.bfloat16), jnp.uint32)


def _unpack(v):
    return pltpu.bitcast(v, jnp.bfloat16)


def _kernel(x_hbm, dw_ref, w1_hbm, w2_hbm, g_ref, b_ref, o_hbm, h_hbm,
            xbuf, hbuf, wc, lhs0, acc, xsem, osem, hsem, *, cfg):
    TM, T, NCACHE, NS, NX = (cfg[k] for k in ("TM", "T", "NCACHE", "NS", "NX"))
    R1, R2, U1, U2 = cfg["R1"], cfg["R2"], cfg["U1"], cfg["U2"]
    F, C = w2_hbm.shape
    CB, FB = C // 3, F // 3
    NSPILL = T - NCACHE - NS
    f32, bf16 = jnp.float32, jnp.bfloat16
    sch1 = sch2 = _HK
    products = range(1, 16)

    def place(t):
        span = T - cfg["TAIL"]
        before = jnp.minimum(t * NCACHE // span, NCACHE)
        ring = jnp.minimum((t + 1) * NCACHE // span, NCACHE) == before
        s = t - before
        return ring, s, jnp.where(ring, s % NS, NS + before)

    def x_load(t):
        return pltpu.make_async_copy(x_hbm.at[pl.ds(t * TM, TM)], xbuf.at[t % NX], xsem.at[t % NX])

    NW = pl.cdiv(F, TM)

    def w2_load(k):
        n, slot = min(TM, F - k * TM), (T + k) % NX
        return pltpu.make_async_copy(w2_hbm.at[pl.ds(k * TM, n)], xbuf.at[slot, pl.ds(0, n)], xsem.at[slot])

    def w2_tile(r0, c0):
        return xbuf[(T + r0 // TM) % NX, r0 % TM:r0 % TM + CB, c0:c0 + CB]

    def o_store(t):
        return pltpu.make_async_copy(xbuf.at[t % NX], o_hbm.at[pl.ds(t * TM, TM)], osem.at[t % NX])

    def h_store(s):
        return pltpu.make_async_copy(hbuf.at[s % NS], h_hbm.at[pl.ds(s * TM, TM)], hsem.at[s % NS])

    def h_load(s):
        return pltpu.make_async_copy(h_hbm.at[pl.ds(s * TM, TM)], hbuf.at[s % NS], hsem.at[s % NS])

    w1_ref = hbuf.at[NS + NCACHE - 1, pl.ds(0, C)]
    w1_load = pltpu.make_async_copy(w1_hbm, w1_ref, hsem.at[0])
    x_load(0).start()
    w1_load.start()
    for t in range(1, U1 + 1):
        x_load(t).start()
    acc[...] = jnp.zeros_like(acc)
    dw = dw_ref[...].astype(f32)

    def layernorm(xs, r0):
        y = xbuf[xs, r0:r0 + R1, :].astype(f32) * dw
        d = y - jnp.sum(y, axis=-1, keepdims=True) * (1.0 / C)
        v = jnp.sum(d * d, axis=-1, keepdims=True) * (1.0 / (C * _BETA ** 2)) + _LN_EPS / _BETA ** 2
        return d * jnp.exp(-0.5 * jnp.log(v))

    def operands1(t, r0):
        rows = [layernorm(t % NX, r0 + i * R1) for i in range(2)]
        a = [[u[:, p * CB:(p + 1) * CB] for p in range(3)] for u in rows]
        return {r: v.astype(bf16) for r, v in _left_operands(sch1, a).items()}

    x_load(0).wait()
    for r, v in operands1(0, 0).items():
        lhs0[r - 1] = v
    w1_load.wait()
    for r in products:
        wc[r - 1] = _pack(_right_operand(
            sch1, r, lambda p, q: w1_ref[p * CB:(p + 1) * CB, q * FB:(q + 1) * FB].astype(f32)))

    def sweep1(it, carry):
        t0 = it * U1
        tiles = [place(t0 + u) for u in range(U1)]
        for u in range(U1):
            @pl.when(t0 + U1 + 1 + u < T)
            def _():
                x_load(t0 + U1 + 1 + u).start()
        for k in range(NW):
            @pl.when(it == (T + k - U1 - 1) // U1)
            def _():
                w2_load(k).start()
        for ring, s, _ in tiles:
            @pl.when(jnp.logical_and(ring, s >= NS))
            def _():
                h_store(s - NS).wait()
        for u in range(1, U1):
            x_load(t0 + u).wait()

        @pl.when(t0 + U1 < T)
        def _():
            x_load(t0 + U1).wait()

        @pl.when(t0 + U1 == T)
        def _():
            w2_load(0).wait()

        per_tile = TM // (2 * R1)
        nsub = U1 * per_tile
        nstream = len(cfg["LAG"])
        SW = FB // nstream
        sumsq = {}

        def product(lhs, c, r):
            return jnp.dot(lhs[r], _unpack(wc[r - 1, :, c * SW:(c + 1) * SW]), preferred_element_type=f32)

        def emit(sub, c, i, q, w):
            h = w * jnp.tanh(w * (w * w + _KAPPA)) + w
            r0, c0 = (sub % per_tile * 2 + i) * R1, q * FB + c * SW
            hbuf[tiles[sub // per_tile][2], r0:r0 + R1, c0:c0 + SW] = h.astype(bf16)
            sq = jnp.sum((h * h).reshape(R1 // 8, 8, SW), axis=0)
            sumsq[c0] = sumsq[c0] + sq if c0 in sumsq else sq

        operands = {0: {r: lhs0[r - 1] for r in products}}

        def left(sub):
            if sub not in operands:
                operands[sub] = operands1(t0 + sub // per_tile, sub % per_tile * 2 * R1)
            return operands[sub]

        def stream(c):
            prev = None
            for sub in range(nsub + 1):
                if sub < nsub:
                    left(sub + 1)
                    cur = _BlockProduct(sch1, functools.partial(product, left(sub), c),
                                        functools.partial(emit, sub, c))
                for r in cfg["ORDER1"]:
                    if r > 0 and sub < nsub:
                        yield cur.step(r)
                    elif r < 0 and prev is not None:
                        yield prev.step(-r)
                prev = cur

        streams = [stream(c) for c in range(nstream)]
        for n in range(15 * nsub + max(cfg["LAG"])):
            for c, lag in enumerate(cfg["LAG"]):
                if 0 <= n - lag < 15 * nsub:
                    next(streams[c])
        for c0, v in sumsq.items():
            acc[:, c0:c0 + SW] += v
        for r, v in left(nsub).items():
            lhs0[r - 1] = v
        for ring, s, _ in tiles:
            @pl.when(jnp.logical_and(ring, s < NSPILL))
            def _():
                h_store(s).start()
        return carry

    jax.lax.fori_loop(0, T // U1, sweep1, 0)

    gx = jnp.sqrt(jnp.sum(acc[...], axis=0, keepdims=True) * _HSCALE ** 2 + _GRN_EPS)
    nx = gx / (jnp.sum(gx, axis=-1, keepdims=True) * (1.0 / F) + _GRN_EPS)
    scale = (g_ref[...].astype(f32) * nx + 1.0) * _HSCALE
    for k in range(1, NW):
        w2_load(k).wait()
    for k in range(FB // CB):
        rows = [p * FB + k * CB for p in range(3)]
        col = [jnp.transpose(jnp.broadcast_to(scale[:, r0:r0 + CB], (CB, CB))) for r0 in rows]
        scaled = [[w2_tile(rows[p], q * CB).astype(f32) * col[p] for q in range(3)] for p in range(3)]
        for r in products:
            wc[r - 1, :, k * CB:(k + 1) * CB] = _pack(_right_operand(sch2, r, lambda p, q: scaled[p][q]))
    w2 = jnp.concatenate([jnp.concatenate([w2_tile(r0, c0) for c0 in range(0, C, CB)], axis=1)
                          for r0 in range(0, F, CB)], axis=0)
    bias = jnp.dot(jnp.broadcast_to(b_ref[...], (16, F)), w2, preferred_element_type=f32)[0:1, :]
    for k in reversed(range(NW)):
        x_load(T - NX + k).start()

    SLACK = cfg["SLACK"]

    def tile2(t):
        ring, s, slot = place(t)

        @pl.when(t + SLACK < T)
        def _():
            o_store(t + SLACK).wait()

            @pl.when(t + SLACK >= NX)
            def _():
                x_load(t + SLACK - NX).start()

        @pl.when(jnp.logical_and(ring, s < NSPILL))
        def _():
            h_load(s).wait()

        @pl.when(t < T - NX + NW)
        def _():
            x_load(t).wait()

        xs = t % NX
        for sub in range(TM // (2 * R2)):
            r0 = sub * 2 * R2
            ops = _left_operands(sch2, [
                [hbuf[slot, r0 + i * R2:r0 + (i + 1) * R2, p * FB:(p + 1) * FB].astype(f32) for p in range(3)]
                for i in range(2)])

            def product(r):
                w = jnp.concatenate(
                    [_unpack(wc[r - 1, :, k * CB:(k + 1) * CB]) for k in range(FB // CB)], axis=0)
                return jnp.dot(ops[r].astype(bf16), w, preferred_element_type=f32)

            def emit(i, q, y):
                rows, cols = slice(r0 + i * R2, r0 + (i + 1) * R2), slice(q * CB, (q + 1) * CB)
                xbuf[xs, rows, cols] = (y + bias[:, cols] + xbuf[xs, rows, cols].astype(f32)).astype(xbuf.dtype)

            bp = _BlockProduct(sch2, product, emit)
            for r in cfg["ORDER2"]:
                bp.step(r)

        o_store(t).start()

        @pl.when(jnp.logical_and(ring, s >= NS))
        def _():
            h_load(s - NS).start()

    def sweep2(it, carry):
        for u in range(U2):
            tile2(T - 1 - it * U2 - u)
        return carry

    jax.lax.fori_loop(0, T // U2, sweep2, 0)
    for t in range(SLACK):
        o_store(t).wait()


_DEFAULT_CFG = dict(
    TM=1024, NCACHE=36, NS=4, TAIL=4, NX=5, SLACK=2, U1=2, U2=2, R1=32, R2=64, VMEM_MB=127.9,
    ORDER1=(7, -6, 11, 8, 9, 2, 14, 10, 4, 12, 5, 15, 1, 3, 13), LAG=(0, 3),
    ORDER2=(7, 8, 9, 10, 4, 11, 12, 3, 15, 5, 2, 14, 13, 1, 6),
)


def _run(x, dw, w1, w2, grn_g, grn_b, cfg):
    B, H, W, C = x.shape
    F = w1.shape[1]
    assert B == 1 and dw.shape[:2] == (1, 1)
    N = H * W
    TM = cfg["TM"]
    T = N // TM
    assert N % TM == 0 and T % cfg["U1"] == 0 and T % cfg["U2"] == 0 and cfg["NX"] > 2 * cfg["U1"]
    cfg = dict(cfg, T=T)
    n_spilled = T - cfg["NCACHE"] - cfg["NS"]
    hbm, vmem = pl.BlockSpec(memory_space=pl.ANY), pl.BlockSpec(memory_space=pltpu.VMEM)
    out, _ = pl.pallas_call(
        functools.partial(_kernel, cfg=cfg),
        in_specs=[hbm, vmem, hbm, hbm, vmem, vmem],
        out_specs=[hbm, hbm],
        out_shape=[
            jax.ShapeDtypeStruct((N, C), x.dtype),
            jax.ShapeDtypeStruct((n_spilled * TM, F), jnp.bfloat16),
        ],
        scratch_shapes=[
            pltpu.VMEM((cfg["NX"], TM, C), x.dtype),
            pltpu.VMEM((cfg["NS"] + cfg["NCACHE"], TM, F), jnp.bfloat16),
            pltpu.VMEM((15, C // 6, F // 3), jnp.uint32),
            pltpu.VMEM((15, cfg["R1"], C // 3), jnp.bfloat16),
            pltpu.VMEM((8, F), jnp.float32),
            pltpu.SemaphoreType.DMA((cfg["NX"],)),
            pltpu.SemaphoreType.DMA((cfg["NX"],)),
            pltpu.SemaphoreType.DMA((cfg["NS"],)),
        ],
        compiler_params=pltpu.CompilerParams(
            vmem_limit_bytes=int(cfg["VMEM_MB"] * 1024 * 1024), flags=cfg.get("FLAGS")),
    )(
        x.reshape(N, C),
        dw.reshape(1, C),
        w1.astype(jnp.bfloat16),
        w2.astype(jnp.bfloat16),
        grn_g.reshape(1, F),
        grn_b.reshape(1, F).astype(jnp.bfloat16),
    )
    return out.reshape(B, H, W, C)


@jax.jit
def pallas_standalone__modern_conv_block_slak__vision_kernel(
    x: jax.Array,
    dw: jax.Array,
    w1: jax.Array,
    w2: jax.Array,
    grn_g: jax.Array,
    grn_b: jax.Array,
):
    return _run(x, dw, w1, w2, grn_g, grn_b, _DEFAULT_CFG)
```

```python
import functools
import math

import jax
import jax.numpy as jnp
import jax.experimental.pallas as pl
import jax.experimental.pallas.tpu as pltpu

_LN_EPS = 1e-5
_GRN_EPS = 1e-6
_C0 = math.sqrt(2.0 / math.pi)
_BETA = (0.044715 * _C0) ** (1.0 / 3.0)
_KAPPA = _C0 / _BETA
_HSCALE = 1.0 / (2.0 * _BETA)

_HK = dict(
    sums={"s1": ("a00", -1, "a10"), "s6": ("a02", -1, "a12"), "s7": ("a00", 1, "a01"), "s8": ("s1", 1, "a01"),
          "s9": ("s8", -1, "a11"), "s10": ("a11", 1, "a12"), "s11": ("a11", -1, "s6"), "s12": ("s11", -1, "a01"),
          "s13": ("a10", 1, "a02"), "s14": ("a10", 1, "a12"), "s15": ("a00", 1, "a02")},
    left={1: "s1", 2: "a10", 3: "a01", 4: "a11", 5: "a02", 6: "s6", 7: "s7", 8: "s8", 9: "s9", 10: "s10",
          11: "s11", 12: "s12", 13: "s13", 14: "s14", 15: "s15"},
    right={
        1: {(0, 0): 1, (0, 2): -1, (1, 0): -1},
        2: {(0, 0): 1, (0, 1): -1, (2, 0): -1},
        3: {(1, 1): 1, (0, 1): -1, (1, 2): -1},
        4: {(1, 1): 1, (1, 0): -1, (2, 1): -1},
        5: {(2, 2): 1, (0, 2): -1, (2, 1): -1},
        6: {(1, 2): 1, (2, 0): 1, (2, 2): -1},
        7: {(0, 1): 1},
        8: {(1, 0): 1, (0, 1): -1},
        9: {(1, 0): -1},
        10: {(2, 1): 1},
        11: {(1, 2): 1, (2, 1): -1},
        12: {(1, 2): -1},
        13: {(2, 0): 1, (0, 2): -1},
        14: {(2, 0): 1},
        15: {(0, 2): 1},
    },
    shared={"q8": ("m7", 1, "m8"), "q9": ("q8", 1, "m9"), "q11": ("m10", 1, "m11"), "q12": ("q11", 1, "m12")},
    outputs={
        (0, 0): {"m1": 1, "m2": 1, "q8": 1, "m13": 1, "m15": 1},
        (0, 1): {"m3": 1, "m7": 1, "q12": 1},
        (0, 2): {"m5": 1, "q12": 1, "m15": 1},
        (1, 0): {"m2": 1, "q9": 1, "m14": 1},
        (1, 1): {"m4": 1, "q9": 1, "m10": 1},
        (1, 2): {"m5": 1, "m6": 1, "q11": 1, "m13": -1, "m14": 1},
    },
)


def _left_operands(scheme, a):
    vals = {"a%d%d" % (i, p): a[i][p] for i in range(2) for p in range(3)}
    for name, (u, sign, v) in scheme["sums"].items():
        vals[name] = vals[u] + vals[v] if sign > 0 else vals[u] - vals[v]
    return {r: vals[name] for r, name in scheme["left"].items()}


def _right_operand(scheme, r, block):
    pos = [block(*pq) for pq, sign in scheme["right"][r].items() if sign > 0]
    neg = [block(*pq) for pq, sign in scheme["right"][r].items() if sign < 0]
    total = functools.reduce(lambda u, v: u + v, pos) if pos else -neg.pop()
    return functools.reduce(lambda u, v: u - v, neg, total)


class _BlockProduct:
    def __init__(self, scheme, product, emit, eager=False):
        self.shared, self.product, self.emit, self.eager = dict(scheme["shared"]), product, emit, eager
        self.ready, self.partial = {}, {}
        self.missing = {iq: dict(terms) for iq, terms in scheme["outputs"].items()}

    def _fold(self, iq, name):
        sign, value = self.missing[iq].pop(name), self.ready[name]
        if iq in self.partial:
            have, total = self.partial[iq]
            if have == sign:
                value = total + value
            else:
                sign, value = 1, (total - value if have > 0 else value - total)
        self.partial[iq] = (sign, value)

    def step(self, r):
        fresh = ["m%d" % r]
        self.ready[fresh[0]] = self.product(r)
        for name, (u, sign, v) in list(self.shared.items()):
            if u in self.ready and v in self.ready:
                self.ready[name] = self.ready[u] + self.ready[v] if sign > 0 else self.ready[u] - self.ready[v]
                fresh.append(name)
                del self.shared[name]
        for iq, terms in list(self.missing.items()):
            if all(name in self.ready for name in terms):
                for name in [n for n in self.ready if n in terms]:
                    self._fold(iq, name)
                self.emit(*iq, self.partial[iq][1])
                del self.missing[iq]
        for name in fresh:
            users = [iq for iq, terms in self.missing.items() if name in terms]
            pending = any(name in (u, v) for u, _, v in self.shared.values())
            if self.eager or (len(users) == 1 and not pending):
                for iq in users:
                    self._fold(iq, name)


def _pack(v):
    return pltpu.bitcast(v.astype(jnp.bfloat16), jnp.uint32)


def _unpack(v):
    return pltpu.bitcast(v, jnp.bfloat16)


def _kernel(x_hbm, dw_ref, w1_hbm, w2_hbm, g_ref, b_ref, o_hbm, h_hbm,
            xbuf, hbuf, wc, lhs0, acc, xsem, osem, hsem, *, cfg):
    TM, T, NCACHE, NS, NX = (cfg[k] for k in ("TM", "T", "NCACHE", "NS", "NX"))
    R1, R2, U1, U2 = cfg["R1"], cfg["R2"], cfg["U1"], cfg["U2"]
    F, C = w2_hbm.shape
    CB, FB = C // 3, F // 3
    NSPILL = T - NCACHE - NS
    f32, bf16 = jnp.float32, jnp.bfloat16
    sch1 = sch2 = _HK
    products = range(1, 16)

    def place(t):
        span = T - cfg["TAIL"]
        before = jnp.minimum(t * NCACHE // span, NCACHE)
        ring = jnp.minimum((t + 1) * NCACHE // span, NCACHE) == before
        s = t - before
        return ring, s, jnp.where(ring, s % NS, NS + before)

    def x_load(t):
        return pltpu.make_async_copy(x_hbm.at[pl.ds(t * TM, TM)], xbuf.at[t % NX, pl.ds(0, TM)], xsem.at[t % NX])

    NW = pl.cdiv(F, TM)

    def w2_load(k):
        n, slot = min(TM, F - k * TM), (T + k) % NX
        return pltpu.make_async_copy(w2_hbm.at[pl.ds(k * TM, n)], xbuf.at[slot, pl.ds(0, n)], xsem.at[slot])

    def w2_tile(r0, c0):
        return xbuf[(T + r0 // TM) % NX, r0 % TM:r0 % TM + CB, c0:c0 + CB]

    def o_store(t):
        return pltpu.make_async_copy(xbuf.at[t % NX, pl.ds(0, TM)], o_hbm.at[pl.ds(t * TM, TM)], osem.at[t % NX])

    def h_store(s):
        return pltpu.make_async_copy(hbuf.at[s % NS], h_hbm.at[pl.ds(s * TM, TM)], hsem.at[s % NS])

    def h_load(s):
        return pltpu.make_async_copy(h_hbm.at[pl.ds(s * TM, TM)], hbuf.at[s % NS], hsem.at[s % NS])

    w1_ref = hbuf.at[NS + NCACHE - 1, pl.ds(0, C)]
    w1_load = pltpu.make_async_copy(w1_hbm, w1_ref, hsem.at[0])
    x_load(0).start()
    w1_load.start()
    for t in range(1, U1 + 1):
        x_load(t).start()
    acc[...] = jnp.zeros_like(acc)
    dw = dw_ref[...].astype(f32)

    def layernorm(xs, r0, n):
        y = xbuf[xs, r0:r0 + n, :].astype(f32) * dw
        d = y - jnp.sum(y, axis=-1, keepdims=True) * (1.0 / C)
        v = jnp.sum(d * d, axis=-1, keepdims=True) + C * _LN_EPS
        return d * jnp.exp2(-0.5 * jnp.log2(v))

    def operands1(rows):
        a = [[u[:, p * CB:(p + 1) * CB] for p in range(3)] for u in rows]
        return {r: v.astype(bf16) for r, v in _left_operands(sch1, a).items()}

    x_load(0).wait()
    AHEAD = cfg["AHEAD"]
    for sub in range(AHEAD):
        for r, v in operands1([layernorm(0, (2 * sub + i) * R1, R1) for i in range(2)]).items():
            lhs0[sub, r - 1] = v
    w1_load.wait()
    for r in products:
        wc[r - 1] = _pack((_BETA * math.sqrt(C)) * _right_operand(
            sch1, r, lambda p, q: w1_ref[p * CB:(p + 1) * CB, q * FB:(q + 1) * FB].astype(f32)))

    def sweep1(it, carry):
        t0 = it * U1
        tiles = [place(t0 + u) for u in range(U1)]
        for u in range(U1):
            @pl.when(t0 + U1 + 1 + u < T)
            def _():
                x_load(t0 + U1 + 1 + u).start()
        for k in range(NW):
            @pl.when(it == (T + k - U1 - 1) // U1)
            def _():
                w2_load(k).start()
        for ring, s, _ in tiles:
            @pl.when(jnp.logical_and(ring, s >= NS))
            def _():
                h_store(s - NS).wait()
        for u in range(1, U1):
            x_load(t0 + u).wait()

        @pl.when(t0 + U1 < T)
        def _():
            x_load(t0 + U1).wait()

        @pl.when(t0 + U1 == T)
        def _():
            w2_load(0).wait()

        per_tile = TM // (2 * R1)
        nsub = U1 * per_tile
        nstream = len(cfg["LAG"])
        SW = FB // nstream
        sumsq = {}

        latest = []

        def product(lhs, c, r):
            latest[:] = [jnp.dot(lhs[r], _unpack(wc[r - 1, :, c * SW:(c + 1) * SW]), preferred_element_type=f32)]
            return latest[0]

        def emit(sub, c, i, q, w):
            h = w * jnp.tanh(w * (w * w + _KAPPA)) + w
            r0, c0 = (sub % per_tile * 2 + i) * R1, q * FB + c * SW
            hbuf[tiles[sub // per_tile][2], r0:r0 + R1, c0:c0 + SW] = h.astype(bf16)
            sq = jnp.sum((h * h).reshape(R1 // 8, 8, SW), axis=0)
            sumsq[c0] = sumsq[c0] + sq if c0 in sumsq else sq

        operands = {sub: {r: lhs0[sub, r - 1] for r in products} for sub in range(AHEAD)}

        gates = cfg["GATES"]
        PR = 2 * R1 // len(gates)

        def norm_piece(sub, k, gated):
            if gated:
                xbuf[(t0 + U1 + 1) % NX, TM:TM + 8, 0:CB] = latest[0][0:8, 0:CB].astype(xbuf.dtype)
            r0 = sub % per_tile * 2 * R1 + k % 2 * R1 + k // 2 * PR
            return layernorm((t0 + sub // per_tile) % NX, r0, PR)

        def stream(c):
            prev = None
            for sub in range(nsub + 1):
                if sub < nsub:
                    cur = _BlockProduct(sch1, functools.partial(product, operands[sub], c),
                                        functools.partial(emit, sub, c), cfg['EAGER1'])
                pieces = {}
                for n, r in enumerate(cfg["ORDER1"]):
                    if r > 0 and sub < nsub:
                        cur.step(r)
                    elif r < 0 and prev is not None:
                        prev.step(-r)
                    if c == 0 and sub < nsub:
                        for k, gate in enumerate(gates):
                            if sub == nsub - 1:
                                gate = min(gate, cfg.get("LASTGATE", -1))
                            if max(gate, 0) == n:
                                pieces[k] = norm_piece(sub + AHEAD, k, gate >= 0)
                    if (r > 0 and sub < nsub) or (r < 0 and prev is not None):
                        yield
                if c == 0 and sub < nsub:
                    operands[sub + AHEAD] = operands1(
                        [jnp.concatenate([pieces[k] for k in range(i, len(gates), 2)], axis=0) for i in range(2)])
                prev = cur

        streams = [stream(c) for c in range(nstream)]
        for n in range(15 * nsub + max(cfg["LAG"])):
            for c, lag in enumerate(cfg["LAG"]):
                if 0 <= n - lag < 15 * nsub:
                    next(streams[c])
        for rest in streams:
            next(rest, None)
        for c0, v in sumsq.items():
            acc[:, c0:c0 + SW] += v
        for sub in range(AHEAD):
            for r, v in operands[nsub + sub].items():
                lhs0[sub, r - 1] = v
        for ring, s, _ in tiles:
            @pl.when(jnp.logical_and(ring, s < NSPILL))
            def _():
                h_store(s).start()
        return carry

    jax.lax.fori_loop(0, T // U1, sweep1, 0)

    gx = jnp.sqrt(jnp.sum(acc[...], axis=0, keepdims=True) * _HSCALE ** 2 + _GRN_EPS)
    nx = gx / (jnp.sum(gx, axis=-1, keepdims=True) * (1.0 / F) + _GRN_EPS)
    scale = (g_ref[...].astype(f32) * nx + 1.0) * _HSCALE
    for k in range(1, NW):
        w2_load(k).wait()
    for k in range(FB // CB):
        rows = [p * FB + k * CB for p in range(3)]
        col = [jnp.transpose(jnp.broadcast_to(scale[:, r0:r0 + CB], (CB, CB))) for r0 in rows]
        scaled = [[w2_tile(rows[p], q * CB).astype(f32) * col[p] for q in range(3)] for p in range(3)]
        for r in products:
            wc[r - 1, :, k * CB:(k + 1) * CB] = _pack(_right_operand(sch2, r, lambda p, q: scaled[p][q]))
    w2 = jnp.concatenate([jnp.concatenate([w2_tile(r0, c0) for c0 in range(0, C, CB)], axis=1)
                          for r0 in range(0, F, CB)], axis=0)
    bias = jnp.dot(jnp.broadcast_to(b_ref[...], (16, F)), w2, preferred_element_type=f32)[0:1, :]
    for k in reversed(range(NW)):
        x_load(T - NX + k).start()

    SLACK = cfg["SLACK"]

    def before(t, ring, s):
        @pl.when(t + SLACK < T)
        def _():
            o_store(t + SLACK).wait()

            @pl.when(t + SLACK >= NX)
            def _():
                x_load(t + SLACK - NX).start()

        @pl.when(jnp.logical_and(ring, s < NSPILL))
        def _():
            h_load(s).wait()

        @pl.when(t < T - NX + NW)
        def _():
            x_load(t).wait()

    def compute(t, slot):
        xs = t % NX
        for sub in range(TM // (2 * R2)):
            r0 = sub * 2 * R2
            ops = _left_operands(sch2, [
                [hbuf[slot, r0 + i * R2:r0 + (i + 1) * R2, p * FB:(p + 1) * FB].astype(f32) for p in range(3)]
                for i in range(2)])

            def product(r):
                w = jnp.concatenate(
                    [_unpack(wc[r - 1, :, k * CB:(k + 1) * CB]) for k in range(FB // CB)], axis=0)
                return jnp.dot(ops[r].astype(bf16), w, preferred_element_type=f32)

            def emit(i, q, y):
                rows, cols = slice(r0 + i * R2, r0 + (i + 1) * R2), slice(q * CB, (q + 1) * CB)
                xbuf[xs, rows, cols] = (y + bias[:, cols] + xbuf[xs, rows, cols].astype(f32)).astype(xbuf.dtype)

            bp = _BlockProduct(sch2, product, emit, cfg['EAGER2'])
            for r in cfg["ORDER2"]:
                bp.step(r)

    def after(t, ring, s):
        o_store(t).start()

        @pl.when(jnp.logical_and(ring, s >= NS))
        def _():
            h_load(s - NS).start()

    def sweep2(it, carry):
        tiles = [T - 1 - it * U2 - u for u in range(U2)]
        tiles = [(t, *place(t)) for t in tiles]
        for t, ring, s, slot in tiles:
            before(t, ring, s)
        for n, (t, ring, s, slot) in enumerate(tiles):
            if not cfg.get('NOCOMP'):
                compute(t, slot)
            if cfg.get("MIDSTART"):
                after(t, ring, s)
        for t, ring, s, slot in tiles:
            if not cfg.get("MIDSTART"):
                after(t, ring, s)
        return carry

    jax.lax.fori_loop(0, T // U2, sweep2, 0)
    for t in range(SLACK):
        o_store(t).wait()


_DEFAULT_CFG = dict(
    TM=1024, NCACHE=36, NS=4, TAIL=4, NX=5, SLACK=2, U1=2, U2=1, R1=32, R2=64, VMEM_MB=127.9,
    ORDER1=(7, 8, 2, 9, 4, 10, 14, 13, 11, 12, 3, 6, 5, 15, 1), LAG=(0, 10), GATES=(4, 7, 9, 11), AHEAD=2,
    EAGER1=1, EAGER2=1,
    ORDER2=(2, 1, 8, 9, 4, 3, 7, 5, 6, 11, 12, 10, 15, 13, 14),
)


def _run(x, dw, w1, w2, grn_g, grn_b, cfg):
    B, H, W, C = x.shape
    F = w1.shape[1]
    assert B == 1 and dw.shape[:2] == (1, 1)
    N = H * W
    TM = cfg["TM"]
    T = N // TM
    assert N % TM == 0 and T % cfg["U1"] == 0 and T % cfg["U2"] == 0 and cfg["NX"] > 2 * cfg["U1"]
    cfg = dict(cfg, T=T)
    n_spilled = T - cfg["NCACHE"] - cfg["NS"]
    hbm, vmem = pl.BlockSpec(memory_space=pl.ANY), pl.BlockSpec(memory_space=pltpu.VMEM)
    out, _ = pl.pallas_call(
        functools.partial(_kernel, cfg=cfg),
        in_specs=[hbm, vmem, hbm, hbm, vmem, vmem],
        out_specs=[hbm, hbm],
        out_shape=[
            jax.ShapeDtypeStruct((N, C), x.dtype),
            jax.ShapeDtypeStruct((n_spilled * TM, F), jnp.bfloat16),
        ],
        scratch_shapes=[
            pltpu.VMEM((cfg["NX"], TM + 16, C), x.dtype),
            pltpu.VMEM((cfg["NS"] + cfg["NCACHE"], TM, F), jnp.bfloat16),
            pltpu.VMEM((15, C // 6, F // 3), jnp.uint32),
            pltpu.VMEM((cfg["AHEAD"], 15, cfg["R1"], C // 3), jnp.bfloat16),
            pltpu.VMEM((8, F), jnp.float32),
            pltpu.SemaphoreType.DMA((cfg["NX"],)),
            pltpu.SemaphoreType.DMA((cfg["NX"],)),
            pltpu.SemaphoreType.DMA((cfg["NS"],)),
        ],
        compiler_params=pltpu.CompilerParams(
            vmem_limit_bytes=int(cfg["VMEM_MB"] * 1024 * 1024), flags=cfg.get("FLAGS")),
    )(
        x.reshape(N, C),
        dw.reshape(1, C),
        w1.astype(jnp.bfloat16),
        w2.astype(jnp.bfloat16),
        grn_g.reshape(1, F),
        grn_b.reshape(1, F).astype(jnp.bfloat16),
    )
    return out.reshape(B, H, W, C)


@jax.jit
def pallas_standalone__modern_conv_block_slak__vision_kernel(
    x: jax.Array,
    dw: jax.Array,
    w1: jax.Array,
    w2: jax.Array,
    grn_g: jax.Array,
    grn_b: jax.Array,
):
    return _run(x, dw, w1, w2, grn_g, grn_b, _DEFAULT_CFG)
```

```python
import functools
import math

import jax
import jax.numpy as jnp
import jax.experimental.pallas as pl
import jax.experimental.pallas.tpu as pltpu

_LN_EPS = 1e-5
_GRN_EPS = 1e-6
_C0 = math.sqrt(2.0 / math.pi)
_BETA = (0.044715 * _C0) ** (1.0 / 3.0)
_KAPPA = _C0 / _BETA
_HSCALE = 1.0 / (2.0 * _BETA)

_HK = dict(
    sums={"s1": ("a00", -1, "a10"), "s6": ("a02", -1, "a12"), "s7": ("a00", 1, "a01"), "s8": ("s1", 1, "a01"),
          "s9": ("s8", -1, "a11"), "s10": ("a11", 1, "a12"), "s11": ("a11", -1, "s6"), "s12": ("s11", -1, "a01"),
          "s13": ("a10", 1, "a02"), "s14": ("a10", 1, "a12"), "s15": ("a00", 1, "a02")},
    left={1: "s1", 2: "a10", 3: "a01", 4: "a11", 5: "a02", 6: "s6", 7: "s7", 8: "s8", 9: "s9", 10: "s10",
          11: "s11", 12: "s12", 13: "s13", 14: "s14", 15: "s15"},
    right={
        1: {(0, 0): 1, (0, 2): -1, (1, 0): -1},
        2: {(0, 0): 1, (0, 1): -1, (2, 0): -1},
        3: {(1, 1): 1, (0, 1): -1, (1, 2): -1},
        4: {(1, 1): 1, (1, 0): -1, (2, 1): -1},
        5: {(2, 2): 1, (0, 2): -1, (2, 1): -1},
        6: {(1, 2): 1, (2, 0): 1, (2, 2): -1},
        7: {(0, 1): 1},
        8: {(1, 0): 1, (0, 1): -1},
        9: {(1, 0): -1},
        10: {(2, 1): 1},
        11: {(1, 2): 1, (2, 1): -1},
        12: {(1, 2): -1},
        13: {(2, 0): 1, (0, 2): -1},
        14: {(2, 0): 1},
        15: {(0, 2): 1},
    },
    shared={"q8": ("m7", 1, "m8"), "q9": ("q8", 1, "m9"), "q11": ("m10", 1, "m11"), "q12": ("q11", 1, "m12")},
    outputs={
        (0, 0): {"m1": 1, "m2": 1, "q8": 1, "m13": 1, "m15": 1},
        (0, 1): {"m3": 1, "m7": 1, "q12": 1},
        (0, 2): {"m5": 1, "q12": 1, "m15": 1},
        (1, 0): {"m2": 1, "q9": 1, "m14": 1},
        (1, 1): {"m4": 1, "q9": 1, "m10": 1},
        (1, 2): {"m5": 1, "m6": 1, "q11": 1, "m13": -1, "m14": 1},
    },
)


def _left_operands(scheme, a):
    vals = {"a%d%d" % (i, p): a[i][p] for i in range(2) for p in range(3)}
    for name, (u, sign, v) in scheme["sums"].items():
        vals[name] = vals[u] + vals[v] if sign > 0 else vals[u] - vals[v]
    return {r: vals[name] for r, name in scheme["left"].items()}


def _right_operand(scheme, r, block):
    pos = [block(*pq) for pq, sign in scheme["right"][r].items() if sign > 0]
    neg = [block(*pq) for pq, sign in scheme["right"][r].items() if sign < 0]
    total = functools.reduce(lambda u, v: u + v, pos) if pos else -neg.pop()
    return functools.reduce(lambda u, v: u - v, neg, total)


class _BlockProduct:
    def __init__(self, scheme, product, emit, eager=False):
        self.shared, self.product, self.emit, self.eager = dict(scheme["shared"]), product, emit, eager
        self.ready, self.partial = {}, {}
        self.missing = {iq: dict(terms) for iq, terms in scheme["outputs"].items()}

    def _fold(self, iq, name):
        sign, value = self.missing[iq].pop(name), self.ready[name]
        if iq in self.partial:
            have, total = self.partial[iq]
            if have == sign:
                value = total + value
            else:
                sign, value = 1, (total - value if have > 0 else value - total)
        self.partial[iq] = (sign, value)

    def step(self, r):
        fresh = ["m%d" % r]
        self.ready[fresh[0]] = self.product(r)
        for name, (u, sign, v) in list(self.shared.items()):
            if u in self.ready and v in self.ready:
                self.ready[name] = self.ready[u] + self.ready[v] if sign > 0 else self.ready[u] - self.ready[v]
                fresh.append(name)
                del self.shared[name]
        for iq, terms in list(self.missing.items()):
            if all(name in self.ready for name in terms):
                for name in [n for n in self.ready if n in terms]:
                    self._fold(iq, name)
                self.emit(*iq, self.partial[iq][1])
                del self.missing[iq]
        for name in fresh:
            users = [iq for iq, terms in self.missing.items() if name in terms]
            pending = any(name in (u, v) for u, _, v in self.shared.values())
            if self.eager or (len(users) == 1 and not pending):
                for iq in users:
                    self._fold(iq, name)


def _pack(v):
    return pltpu.bitcast(v.astype(jnp.bfloat16), jnp.uint32)


def _unpack(v):
    return pltpu.bitcast(v, jnp.bfloat16)


def _kernel(x_hbm, dw_ref, w1_hbm, w2_hbm, g_ref, b_ref, o_hbm, h_hbm,
            xbuf, hbuf, wc, lhs0, acc, xsem, osem, hsem, *, cfg):
    TM, T, NCACHE, NS, NX = (cfg[k] for k in ("TM", "T", "NCACHE", "NS", "NX"))
    R1, R2, U1 = cfg["R1"], cfg["R2"], cfg["U1"]
    F, C = w2_hbm.shape
    CB, FB = C // 3, F // 3
    NSPILL = T - NCACHE - NS
    f32, bf16 = jnp.float32, jnp.bfloat16
    sch1 = sch2 = _HK
    products = range(1, 16)

    def place(t):
        span = T - cfg["TAIL"]
        before = jnp.minimum(t * NCACHE // span, NCACHE)
        ring = jnp.minimum((t + 1) * NCACHE // span, NCACHE) == before
        s = t - before
        return ring, s, jnp.where(ring, s % NS, NS + before)

    def x_load(t):
        return pltpu.make_async_copy(x_hbm.at[pl.ds(t * TM, TM)], xbuf.at[t % NX, pl.ds(0, TM)], xsem.at[t % NX])

    NW = pl.cdiv(F, TM)

    def w2_load(k):
        n, slot = min(TM, F - k * TM), (T + k) % NX
        return pltpu.make_async_copy(w2_hbm.at[pl.ds(k * TM, n)], xbuf.at[slot, pl.ds(0, n)], xsem.at[slot])

    def w2_tile(r0, c0):
        return xbuf[(T + r0 // TM) % NX, r0 % TM:r0 % TM + CB, c0:c0 + CB]

    def o_store(t):
        return pltpu.make_async_copy(xbuf.at[t % NX, pl.ds(0, TM)], o_hbm.at[pl.ds(t * TM, TM)], osem.at[t % NX])

    def h_store(s):
        return pltpu.make_async_copy(hbuf.at[s % NS], h_hbm.at[s], hsem.at[s % NS])

    def h_load(s):
        return pltpu.make_async_copy(h_hbm.at[s], hbuf.at[s % NS], hsem.at[s % NS])

    w1_loads = [pltpu.make_async_copy(w1_hbm.at[:, pl.ds(j * CB, CB)], hbuf.at[NS + NCACHE - 1, j, pl.ds(0, C)],
                                      hsem.at[0]) for j in range(F // CB)]
    x_load(0).start()
    for load in w1_loads:
        load.start()

    def h_block(slot, r0, n, p):
        return jnp.concatenate([hbuf[slot, p * (FB // CB) + k, r0:r0 + n, :].astype(f32)
                                for k in range(FB // CB)], axis=1)

    for t in range(1, U1 + 1):
        x_load(t).start()
    acc[...] = jnp.zeros_like(acc)
    dw = dw_ref[...].astype(f32)

    def layernorm(xs, r0, n):
        y = xbuf[xs, r0:r0 + n, :].astype(f32) * dw
        d = y - jnp.sum(y, axis=-1, keepdims=True) * (1.0 / C)
        v = jnp.sum(d * d, axis=-1, keepdims=True) + C * _LN_EPS
        return d * jnp.exp2(-0.5 * jnp.log2(v))

    def operands1(rows):
        a = [[u[:, p * CB:(p + 1) * CB] for p in range(3)] for u in rows]
        return {r: v.astype(bf16) for r, v in _left_operands(sch1, a).items()}

    x_load(0).wait()
    AHEAD = cfg["AHEAD"]
    for sub in range(AHEAD):
        for r, v in operands1([layernorm(0, (2 * sub + i) * R1, R1) for i in range(2)]).items():
            lhs0[sub, r - 1] = v
    for load in w1_loads:
        load.wait()
    for r in products[:cfg.get("NPREP")]:
        wc[r - 1] = _pack((_BETA * math.sqrt(C)) * _right_operand(
            sch1, r, lambda p, q: h_block(NS + NCACHE - 1, p * CB, CB, q)))

    def places(t0, step, n):
        return [place(t0 + step * u) for u in range(n)]

    def sweep1(it, carry):
        t0 = it * U1
        done, tiles = carry
        for ring, s, _ in tiles:
            @pl.when(jnp.logical_and(ring, s >= NS))
            def _():
                h_store(s - NS).wait()
        for u in range(1, U1):
            x_load(t0 + u).wait()

        @pl.when(t0 + U1 < T)
        def _():
            x_load(t0 + U1).wait()

        @pl.when(t0 + U1 == T)
        def _():
            w2_load(0).wait()

        def start_copies():
            for ring, s, _ in done:
                @pl.when(jnp.logical_and(ring, s < NSPILL))
                def _():
                    h_store(s).start()
            for u in range(U1):
                @pl.when(t0 + U1 + 1 + u < T)
                def _():
                    x_load(t0 + U1 + 1 + u).start()
            for k in range(NW):
                @pl.when(it == (T + k - U1 - 1) // U1)
                def _():
                    w2_load(k).start()

        per_tile = TM // (2 * R1)
        nsub = U1 * per_tile
        nstream = len(cfg["LAG"])
        SW = FB // nstream
        sumsq = {}

        latest = []

        def product(lhs, c, r):
            latest[:] = [jnp.dot(lhs[r], _unpack(wc[r - 1, :, c * SW:(c + 1) * SW]), preferred_element_type=f32)]
            return latest[0]

        def emit(sub, c, i, q, w):
            h = w * jnp.tanh(w * (w * w + _KAPPA)) + w
            r0, c0 = (sub % per_tile * 2 + i) * R1, q * FB + c * SW
            for k in range(SW // CB):
                hbuf[tiles[sub // per_tile][2], c0 // CB + k, r0:r0 + R1, :] = h[:, k * CB:(k + 1) * CB].astype(bf16)
            sq = jnp.sum((h * h).reshape(R1 // 8, 8, SW), axis=0)
            sumsq[c0] = sumsq[c0] + sq if c0 in sumsq else sq

        operands = {sub: {r: lhs0[sub, r - 1] for r in products} for sub in range(AHEAD)}

        gates = cfg["GATES"]
        PR = 2 * R1 // len(gates)

        def norm_piece(sub, k, gated):
            if gated:
                xbuf[(t0 + U1 + 1) % NX, TM:TM + 8, 0:CB] = latest[0][0:8, 0:CB].astype(xbuf.dtype)
            r0 = sub % per_tile * 2 * R1 + k % 2 * R1 + k // 2 * PR
            return layernorm((t0 + sub // per_tile) % NX, r0, PR)

        def stream(c):
            prev = None
            for sub in range(nsub + 1):
                if sub < nsub:
                    cur = _BlockProduct(sch1, functools.partial(product, operands[sub], c),
                                        functools.partial(emit, sub, c), cfg['EAGER1'])
                pieces = {}
                for n, r in enumerate(cfg["ORDER1"]):
                    if r > 0 and sub < nsub:
                        cur.step(r)
                    elif r < 0 and prev is not None:
                        prev.step(-r)
                    if c == 0 and sub < nsub:
                        for k, gate in enumerate(gates):
                            if sub == nsub - 1:
                                gate = min(gate, cfg.get("LASTGATE", -1))
                            if max(gate, 0) == n:
                                pieces[k] = norm_piece(sub + AHEAD, k, gate >= 0)
                    if (r > 0 and sub < nsub) or (r < 0 and prev is not None):
                        yield
                if c == 0 and sub < nsub:
                    operands[sub + AHEAD] = operands1(
                        [jnp.concatenate([pieces[k] for k in range(i, len(gates), 2)], axis=0) for i in range(2)])
                prev = cur

        streams = [stream(c) for c in range(nstream)]
        for n in range(15 * nsub + max(cfg["LAG"])):
            for c, lag in enumerate(cfg["LAG"]):
                if 0 <= n - lag < 15 * nsub:
                    next(streams[c])
            if n == cfg["START1"]:
                start_copies()
        for rest in streams:
            next(rest, None)
        for c0, v in sumsq.items():
            acc[:, c0:c0 + SW] += v
        for sub in range(AHEAD):
            for r, v in operands[nsub + sub].items():
                lhs0[sub, r - 1] = v
        return tiles, places(t0 + U1, 1, U1)

    first = places(jnp.int32(0), 1, U1)
    nothing = [(jnp.logical_and(ring, False), s, slot) for ring, s, slot in first]
    jax.lax.fori_loop(0, T // U1, sweep1, (nothing, first))

    gx = jnp.sqrt(jnp.sum(acc[...], axis=0, keepdims=True) * _HSCALE ** 2 + _GRN_EPS)
    nx = gx / (jnp.sum(gx, axis=-1, keepdims=True) * (1.0 / F) + _GRN_EPS)
    scale = (g_ref[...].astype(f32) * nx + 1.0) * _HSCALE
    for k in range(1, NW):
        w2_load(k).wait()
    for k in range(FB // CB):
        rows = [p * FB + k * CB for p in range(3)]
        col = [jnp.transpose(jnp.broadcast_to(scale[:, r0:r0 + CB], (CB, CB))) for r0 in rows]
        scaled = [[w2_tile(rows[p], q * CB).astype(f32) * col[p] for q in range(3)] for p in range(3)]
        for r in products:
            wc[r - 1, :, k * CB:(k + 1) * CB] = _pack(_right_operand(sch2, r, lambda p, q: scaled[p][q]))
    w2 = jnp.concatenate([jnp.concatenate([w2_tile(r0, c0) for c0 in range(0, C, CB)], axis=1)
                          for r0 in range(0, F, CB)], axis=0)
    bias = jnp.dot(jnp.broadcast_to(b_ref[...], (16, F)), w2, preferred_element_type=f32)[0:1, :]
    for k in reversed(range(NW)):
        x_load(T - NX + k).start()

    SLACK = cfg["SLACK"]

    def compute(t, slot, hook):
        xs = t % NX
        for sub in range(TM // (2 * R2)):
            r0 = sub * 2 * R2
            ops = _left_operands(sch2, [
                [h_block(slot, r0 + i * R2, R2, p) for p in range(3)] for i in range(2)])

            def product(r):
                w = jnp.concatenate(
                    [_unpack(wc[r - 1, :, k * CB:(k + 1) * CB]) for k in range(FB // CB)], axis=0)
                return jnp.dot(ops[r].astype(bf16), w, preferred_element_type=f32)

            def emit(i, q, y):
                rows, cols = slice(r0 + i * R2, r0 + (i + 1) * R2), slice(q * CB, (q + 1) * CB)
                xbuf[xs, rows, cols] = (y + bias[:, cols] + xbuf[xs, rows, cols].astype(f32)).astype(xbuf.dtype)

            bp = _BlockProduct(sch2, product, emit, cfg['EAGER2'])
            for n, r in enumerate(cfg["ORDER2"]):
                bp.step(r)
                if (sub, n) == cfg["HOOK"]:
                    hook()

    def sweep2(step, carry):
        t = T - 1 - step
        (done_ring, done_s, _), (ring, s, slot) = carry

        @pl.when(t + SLACK < T)
        def _():
            o_store(t + SLACK).wait()

        @pl.when(jnp.logical_and(ring, s < NSPILL))
        def _():
            h_load(s).wait()

        @pl.when(t < T - NX + NW)
        def _():
            x_load(t).wait()

        def start_copies():
            @pl.when(step > 0)
            def _():
                o_store(t + 1).start()

            @pl.when(jnp.logical_and(done_ring, done_s >= NS))
            def _():
                h_load(done_s - NS).start()

            @pl.when(jnp.logical_and(t + SLACK < T, t + SLACK >= NX))
            def _():
                x_load(t + SLACK - NX).start()

        compute(t, slot, start_copies)
        return (ring, s, slot), place(jnp.maximum(t - 1, 0))

    last = place(jnp.int32(T - 1))
    jax.lax.fori_loop(0, T, sweep2, ((jnp.logical_and(last[0], False), *last[1:]), last))
    o_store(0).start()
    for t in range(SLACK):
        o_store(t).wait()


_DEFAULT_CFG = dict(
    TM=1024, NCACHE=36, NS=4, TAIL=4, NX=5, SLACK=2, U1=2, U2=1, R1=32, R2=64, VMEM_MB=127.9,
    ORDER1=(8, 7, 2, 9, 4, 10, 14, 6, 13, 11, 12, 3, 5, 15, 1), LAG=(0, 0, 10, 11), GATES=(2, 4, 7, 11), AHEAD=2,
    EAGER1=1, EAGER2=1, HOOK=(0, 1), START1=2,
    ORDER2=(2, 1, 8, 9, 4, 3, 7, 5, 6, 11, 12, 10, 15, 13, 14),
)


def _run(x, dw, w1, w2, grn_g, grn_b, cfg):
    B, H, W, C = x.shape
    F = w1.shape[1]
    assert B == 1 and dw.shape[:2] == (1, 1)
    N = H * W
    TM = cfg["TM"]
    T = N // TM
    assert N % TM == 0 and T % cfg["U1"] == 0 and cfg["NX"] > 2 * cfg["U1"]
    cfg = dict(cfg, T=T)
    n_spilled = T - cfg["NCACHE"] - cfg["NS"]
    hbm, vmem = pl.BlockSpec(memory_space=pl.ANY), pl.BlockSpec(memory_space=pltpu.VMEM)
    out, _ = pl.pallas_call(
        functools.partial(_kernel, cfg=cfg),
        in_specs=[hbm, vmem, hbm, hbm, vmem, vmem],
        out_specs=[hbm, hbm],
        out_shape=[
            jax.ShapeDtypeStruct((N, C), x.dtype),
            jax.ShapeDtypeStruct((n_spilled, F // 128, TM, 128), jnp.bfloat16),
        ],
        scratch_shapes=[
            pltpu.VMEM((cfg["NX"], TM + 16, C), x.dtype),
            pltpu.VMEM((cfg["NS"] + cfg["NCACHE"], F // 128, TM, 128), jnp.bfloat16),
            pltpu.VMEM((15, C // 6, F // 3), jnp.uint32),
            pltpu.VMEM((cfg["AHEAD"], 15, cfg["R1"], C // 3), jnp.bfloat16),
            pltpu.VMEM((8, F), jnp.float32),
            pltpu.SemaphoreType.DMA((cfg["NX"],)),
            pltpu.SemaphoreType.DMA((cfg["NX"],)),
            pltpu.SemaphoreType.DMA((cfg["NS"],)),
        ],
        compiler_params=pltpu.CompilerParams(
            vmem_limit_bytes=int(cfg["VMEM_MB"] * 1024 * 1024), flags=cfg.get("FLAGS")),
    )(
        x.reshape(N, C),
        dw.reshape(1, C),
        w1.astype(jnp.bfloat16),
        w2.astype(jnp.bfloat16),
        grn_g.reshape(1, F),
        grn_b.reshape(1, F).astype(jnp.bfloat16),
    )
    return out.reshape(B, H, W, C)


@jax.jit
def pallas_standalone__modern_conv_block_slak__vision_kernel(
    x: jax.Array,
    dw: jax.Array,
    w1: jax.Array,
    w2: jax.Array,
    grn_g: jax.Array,
    grn_b: jax.Array,
):
    return _run(x, dw, w1, w2, grn_g, grn_b, _DEFAULT_CFG)
```

```python
import functools
import math

import jax
import jax.numpy as jnp
import jax.experimental.pallas as pl
import jax.experimental.pallas.tpu as pltpu

_LN_EPS = 1e-5
_GRN_EPS = 1e-6
_C0 = math.sqrt(2.0 / math.pi)
_BETA = (0.044715 * _C0) ** (1.0 / 3.0)
_KAPPA = _C0 / _BETA
_HSCALE = 1.0 / (2.0 * _BETA)

_HK = dict(
    sums={"s1": ("a00", -1, "a10"), "s6": ("a02", -1, "a12"), "s7": ("a00", 1, "a01"), "s8": ("s1", 1, "a01"),
          "s9": ("s8", -1, "a11"), "s10": ("a11", 1, "a12"), "s11": ("a11", -1, "s6"), "s12": ("s11", -1, "a01"),
          "s13": ("a10", 1, "a02"), "s14": ("a10", 1, "a12"), "s15": ("a00", 1, "a02")},
    left={1: "s1", 2: "a10", 3: "a01", 4: "a11", 5: "a02", 6: "s6", 7: "s7", 8: "s8", 9: "s9", 10: "s10",
          11: "s11", 12: "s12", 13: "s13", 14: "s14", 15: "s15"},
    right={
        1: {(0, 0): 1, (0, 2): -1, (1, 0): -1},
        2: {(0, 0): 1, (0, 1): -1, (2, 0): -1},
        3: {(1, 1): 1, (0, 1): -1, (1, 2): -1},
        4: {(1, 1): 1, (1, 0): -1, (2, 1): -1},
        5: {(2, 2): 1, (0, 2): -1, (2, 1): -1},
        6: {(1, 2): 1, (2, 0): 1, (2, 2): -1},
        7: {(0, 1): 1},
        8: {(1, 0): 1, (0, 1): -1},
        9: {(1, 0): -1},
        10: {(2, 1): 1},
        11: {(1, 2): 1, (2, 1): -1},
        12: {(1, 2): -1},
        13: {(2, 0): 1, (0, 2): -1},
        14: {(2, 0): 1},
        15: {(0, 2): 1},
    },
    shared={"q8": ("m7", 1, "m8"), "q9": ("q8", 1, "m9"), "q11": ("m10", 1, "m11"), "q12": ("q11", 1, "m12")},
    outputs={
        (0, 0): {"m1": 1, "m2": 1, "q8": 1, "m13": 1, "m15": 1},
        (0, 1): {"m3": 1, "m7": 1, "q12": 1},
        (0, 2): {"m5": 1, "q12": 1, "m15": 1},
        (1, 0): {"m2": 1, "q9": 1, "m14": 1},
        (1, 1): {"m4": 1, "q9": 1, "m10": 1},
        (1, 2): {"m5": 1, "m6": 1, "q11": 1, "m13": -1, "m14": 1},
    },
)


def _left_operands(scheme, a):
    vals = {"a%d%d" % (i, p): a[i][p] for i in range(2) for p in range(3)}
    for name, (u, sign, v) in scheme["sums"].items():
        vals[name] = vals[u] + vals[v] if sign > 0 else vals[u] - vals[v]
    return {r: vals[name] for r, name in scheme["left"].items()}


def _right_operand(scheme, r, block):
    pos = [block(*pq) for pq, sign in scheme["right"][r].items() if sign > 0]
    neg = [block(*pq) for pq, sign in scheme["right"][r].items() if sign < 0]
    total = functools.reduce(lambda u, v: u + v, pos) if pos else -neg.pop()
    return functools.reduce(lambda u, v: u - v, neg, total)


class _BlockProduct:
    def __init__(self, scheme, product, emit, eager=False):
        self.shared, self.product, self.emit, self.eager = dict(scheme["shared"]), product, emit, eager
        self.ready, self.partial = {}, {}
        self.missing = {iq: dict(terms) for iq, terms in scheme["outputs"].items()}

    def _fold(self, iq, name):
        sign, value = self.missing[iq].pop(name), self.ready[name]
        if iq in self.partial:
            have, total = self.partial[iq]
            if have == sign:
                value = total + value
            else:
                sign, value = 1, (total - value if have > 0 else value - total)
        self.partial[iq] = (sign, value)

    def step(self, r):
        fresh = ["m%d" % r]
        self.ready[fresh[0]] = self.product(r)
        for name, (u, sign, v) in list(self.shared.items()):
            if u in self.ready and v in self.ready:
                self.ready[name] = self.ready[u] + self.ready[v] if sign > 0 else self.ready[u] - self.ready[v]
                fresh.append(name)
                del self.shared[name]
        for iq, terms in list(self.missing.items()):
            if all(name in self.ready for name in terms):
                for name in [n for n in self.ready if n in terms]:
                    self._fold(iq, name)
                self.emit(*iq, self.partial[iq][1])
                del self.missing[iq]
        for name in fresh:
            users = [iq for iq, terms in self.missing.items() if name in terms]
            pending = any(name in (u, v) for u, _, v in self.shared.values())
            if self.eager or (len(users) == 1 and not pending):
                for iq in users:
                    self._fold(iq, name)


def _pack(v):
    return pltpu.bitcast(v.astype(jnp.bfloat16), jnp.uint32)


def _unpack(v):
    return pltpu.bitcast(v, jnp.bfloat16)


def _kernel(x_hbm, dw_ref, w1_hbm, w2_hbm, g_ref, b_ref, o_hbm, h_hbm,
            xbuf, hbuf, wc, lhs0, acc, xsem, osem, hsem, *, cfg):
    TM, T, NCACHE, NS, NX = (cfg[k] for k in ("TM", "T", "NCACHE", "NS", "NX"))
    R1, R2, U1 = cfg["R1"], cfg["R2"], cfg["U1"]
    F, C = w2_hbm.shape
    CB, FB = C // 3, F // 3
    NSPILL = T - NCACHE - NS
    f32, bf16 = jnp.float32, jnp.bfloat16
    sch1 = sch2 = _HK
    products = range(1, 16)

    def place(t):
        span = T - cfg["TAIL"]
        before = jnp.minimum(t * NCACHE // span, NCACHE)
        ring = jnp.minimum((t + 1) * NCACHE // span, NCACHE) == before
        s = t - before
        return ring, s, jnp.where(ring, s % NS, NS + before)

    def x_load(t):
        return pltpu.make_async_copy(x_hbm.at[pl.ds(t * TM, TM)], xbuf.at[t % NX, pl.ds(0, TM)], xsem.at[t % NX])

    NW = pl.cdiv(F, TM)

    def w2_load(k):
        n, slot = min(TM, F - k * TM), (T + k) % NX
        return pltpu.make_async_copy(w2_hbm.at[pl.ds(k * TM, n)], xbuf.at[slot, pl.ds(0, n)], xsem.at[slot])

    def w2_tile(r0, c0):
        return xbuf[(T + r0 // TM) % NX, r0 % TM:r0 % TM + CB, c0:c0 + CB]

    def o_store(t):
        return pltpu.make_async_copy(xbuf.at[t % NX, pl.ds(0, TM)], o_hbm.at[pl.ds(t * TM, TM)], osem.at[t % NX])

    def h_store(s):
        return pltpu.make_async_copy(hbuf.at[s % NS], h_hbm.at[s], hsem.at[s % NS])

    def h_load(s):
        return pltpu.make_async_copy(h_hbm.at[s], hbuf.at[s % NS], hsem.at[s % NS])

    w1_loads = [pltpu.make_async_copy(w1_hbm.at[:, pl.ds(j * CB, CB)], hbuf.at[NS + NCACHE - 1, j, pl.ds(0, C)],
                                      hsem.at[0]) for j in range(F // CB)]
    x_load(0).start()
    for load in w1_loads:
        load.start()

    def h_block(slot, r0, n, p):
        return jnp.concatenate([hbuf[slot, p * (FB // CB) + k, r0:r0 + n, :].astype(f32)
                                for k in range(FB // CB)], axis=1)

    for t in range(1, U1 + 1):
        x_load(t).start()
    acc[...] = jnp.zeros_like(acc)
    dw = dw_ref[...].astype(f32)

    def layernorm(xs, r0, n):
        y = xbuf[xs, r0:r0 + n, :].astype(f32) * dw
        d = y - jnp.sum(y, axis=-1, keepdims=True) * (1.0 / C)
        v = jnp.sum(d * d, axis=-1, keepdims=True) + C * _LN_EPS
        return d * jnp.exp2(-0.5 * jnp.log2(v))

    def operands1(rows):
        a = [[u[:, p * CB:(p + 1) * CB] for p in range(3)] for u in rows]
        return {r: v.astype(bf16) for r, v in _left_operands(sch1, a).items()}

    x_load(0).wait()
    AHEAD = cfg["AHEAD"]
    for sub in range(AHEAD):
        for r, v in operands1([layernorm(0, (2 * sub + i) * R1, R1) for i in range(2)]).items():
            lhs0[sub, r - 1] = v
    for load in w1_loads:
        load.wait()
    for r in products[:cfg.get("NPREP")]:
        wc[r - 1] = _pack((_BETA * math.sqrt(C)) * _right_operand(
            sch1, r, lambda p, q: h_block(NS + NCACHE - 1, p * CB, CB, q)))

    def places(t0, step, n):
        return [place(t0 + step * u) for u in range(n)]

    def sweep1(it, carry):
        t0 = it * U1
        done, tiles = carry
        for ring, s, _ in tiles:
            @pl.when(jnp.logical_and(ring, s >= NS))
            def _():
                h_store(s - NS).wait()
        for u in range(1, U1):
            x_load(t0 + u).wait()

        @pl.when(t0 + U1 < T)
        def _():
            x_load(t0 + U1).wait()

        @pl.when(t0 + U1 == T)
        def _():
            w2_load(0).wait()

        def start_copies():
            for ring, s, _ in done:
                @pl.when(jnp.logical_and(ring, s < NSPILL))
                def _():
                    h_store(s).start()
            for u in range(U1):
                @pl.when(t0 + U1 + 1 + u < T)
                def _():
                    x_load(t0 + U1 + 1 + u).start()
            for k in range(NW):
                @pl.when(it == (T + k - U1 - 1) // U1)
                def _():
                    w2_load(k).start()

        per_tile = TM // (2 * R1)
        nsub = U1 * per_tile
        nstream = len(cfg["LAG"])
        SW = FB // nstream
        sumsq = {}

        latest = []

        def product(lhs, c, r):
            latest[:] = [jnp.dot(lhs[r], _unpack(wc[r - 1, :, c * SW:(c + 1) * SW]), preferred_element_type=f32)]
            return latest[0]

        def emit(sub, c, i, q, w):
            h = w * jnp.tanh(w * (w * w + _KAPPA)) + w
            r0, c0 = (sub % per_tile * 2 + i) * R1, q * FB + c * SW
            for k in range(SW // CB):
                hbuf[tiles[sub // per_tile][2], c0 // CB + k, r0:r0 + R1, :] = h[:, k * CB:(k + 1) * CB].astype(bf16)
            sq = jnp.sum((h * h).reshape(R1 // 8, 8, SW), axis=0)
            sumsq[c0] = sumsq[c0] + sq if c0 in sumsq else sq

        operands = {sub: {r: lhs0[sub, r - 1] for r in products} for sub in range(AHEAD)}

        gates = cfg["GATES"]
        PR = 2 * R1 // len(gates)

        def norm_piece(sub, k, gated):
            if gated:
                xbuf[(t0 + U1 + 1) % NX, TM:TM + 8, 0:CB] = latest[0][0:8, 0:CB].astype(xbuf.dtype)
            r0 = sub % per_tile * 2 * R1 + k % 2 * R1 + k // 2 * PR
            return layernorm((t0 + sub // per_tile) % NX, r0, PR)

        def stream(c):
            prev = None
            for sub in range(nsub + 1):
                if sub < nsub:
                    cur = _BlockProduct(sch1, functools.partial(product, operands[sub], c),
                                        functools.partial(emit, sub, c), cfg['EAGER1'])
                pieces = {}
                order = cfg["ORDER1"] if 2 * c < nstream else cfg.get("ORDER1B", cfg["ORDER1"])
                for n, r in enumerate(order):
                    if r > 0 and sub < nsub:
                        cur.step(r)
                    elif r < 0 and prev is not None:
                        prev.step(-r)
                    if c == 0 and sub < nsub:
                        for k, gate in enumerate(gates):
                            if sub == nsub - 1:
                                gate = min(gate, cfg.get("LASTGATE", -1))
                            if max(gate, 0) == n:
                                pieces[k] = norm_piece(sub + AHEAD, k, gate >= 0)
                    if (r > 0 and sub < nsub) or (r < 0 and prev is not None):
                        yield
                if c == 0 and sub < nsub:
                    operands[sub + AHEAD] = operands1(
                        [jnp.concatenate([pieces[k] for k in range(i, len(gates), 2)], axis=0) for i in range(2)])
                prev = cur

        streams = [stream(c) for c in range(nstream)]
        for n in range(15 * nsub + max(cfg["LAG"])):
            for c, lag in enumerate(cfg["LAG"]):
                if 0 <= n - lag < 15 * nsub:
                    next(streams[c])
            if n == cfg["START1"]:
                start_copies()
        for rest in streams:
            next(rest, None)
        for c0, v in sumsq.items():
            acc[:, c0:c0 + SW] += v
        for sub in range(AHEAD):
            for r, v in operands[nsub + sub].items():
                lhs0[sub, r - 1] = v
        return tiles, places(t0 + U1, 1, U1)

    first = places(jnp.int32(0), 1, U1)
    nothing = [(jnp.logical_and(ring, False), s, slot) for ring, s, slot in first]
    jax.lax.fori_loop(0, T // U1, sweep1, (nothing, first))

    gx = jnp.sqrt(jnp.sum(acc[...], axis=0, keepdims=True) * _HSCALE ** 2 + _GRN_EPS)
    nx = gx / (jnp.sum(gx, axis=-1, keepdims=True) * (1.0 / F) + _GRN_EPS)
    scale = (g_ref[...].astype(f32) * nx + 1.0) * _HSCALE
    for k in range(1, NW):
        w2_load(k).wait()
    for k in range(FB // CB):
        rows = [p * FB + k * CB for p in range(3)]
        col = [jnp.transpose(jnp.broadcast_to(scale[:, r0:r0 + CB], (CB, CB))) for r0 in rows]
        scaled = [[w2_tile(rows[p], q * CB).astype(f32) * col[p] for q in range(3)] for p in range(3)]
        for r in products:
            wc[r - 1, :, k * CB:(k + 1) * CB] = _pack(_right_operand(sch2, r, lambda p, q: scaled[p][q]))
    w2 = jnp.concatenate([jnp.concatenate([w2_tile(r0, c0) for c0 in range(0, C, CB)], axis=1)
                          for r0 in range(0, F, CB)], axis=0)
    bias = jnp.dot(jnp.broadcast_to(b_ref[...], (16, F)), w2, preferred_element_type=f32)[0:1, :]
    for k in reversed(range(NW)):
        x_load(T - NX + k).start()

    SLACK = cfg["SLACK"]

    def compute(t, slot, hook):
        xs = t % NX
        for sub in range(TM // (2 * R2)):
            r0 = sub * 2 * R2
            ops = _left_operands(sch2, [
                [h_block(slot, r0 + i * R2, R2, p) for p in range(3)] for i in range(2)])

            def product(r):
                w = jnp.concatenate(
                    [_unpack(wc[r - 1, :, k * CB:(k + 1) * CB]) for k in range(FB // CB)], axis=0)
                return jnp.dot(ops[r].astype(bf16), w, preferred_element_type=f32)

            def emit(i, q, y):
                rows, cols = slice(r0 + i * R2, r0 + (i + 1) * R2), slice(q * CB, (q + 1) * CB)
                xbuf[xs, rows, cols] = (y + bias[:, cols] + xbuf[xs, rows, cols].astype(f32)).astype(xbuf.dtype)

            bp = _BlockProduct(sch2, product, emit, cfg['EAGER2'])
            for n, r in enumerate(cfg["ORDER2"]):
                bp.step(r)
                if (sub, n) == cfg["HOOK"]:
                    hook()

    def sweep2(step, carry):
        t = T - 1 - step
        (done_ring, done_s, _), (ring, s, slot) = carry

        def release():
            @pl.when(jnp.logical_and(done_ring, done_s >= NS))
            def _():
                h_load(done_s - NS).start()

            @pl.when(step > 0)
            def _():
                o_store(t + 1).start()

        if cfg["EARLY"]:
            release()

        @pl.when(t + SLACK < T)
        def _():
            o_store(t + SLACK).wait()

        def refill():
            @pl.when(jnp.logical_and(t + SLACK < T, t + SLACK >= NX))
            def _():
                x_load(t + SLACK - NX).start()

        if cfg["EARLY"] > 1:
            refill()

        @pl.when(jnp.logical_and(ring, s < NSPILL))
        def _():
            h_load(s).wait()

        @pl.when(t < T - NX + NW)
        def _():
            x_load(t).wait()

        def start_copies():
            if not cfg["EARLY"]:
                release()
            if cfg["EARLY"] < 2:
                refill()

        compute(t, slot, start_copies)
        return (ring, s, slot), place(jnp.maximum(t - 1, 0))

    last = place(jnp.int32(T - 1))
    jax.lax.fori_loop(0, T, sweep2, ((jnp.logical_and(last[0], False), *last[1:]), last))
    o_store(0).start()
    for t in range(SLACK):
        o_store(t).wait()


_DEFAULT_CFG = dict(
    TM=1024, NCACHE=36, NS=4, TAIL=4, NX=5, SLACK=2, U1=2, U2=1, R1=32, R2=64, VMEM_MB=127.9,
    ORDER1=(8, 9, 7, 4, 2, 14, 10, 6, 13, 11, 12, 3, 5, 15, 1), ORDER1B=(8, 7, 2, 9, 10, 4, 14, 6, 13, 11, 12, 3, 5, 15, 1),
    LAG=(0, 0, 10, 11), GATES=(1, 2, 4, 5, 6, 8, 10, 11), AHEAD=2,
    EAGER1=1, EAGER2=1, HOOK=(0, 1), START1=2, EARLY=0, NOBC=1,
    ORDER2=(5, 2, 1, 8, 9, 7, 4, 3, 6, 11, 10, 13, 12, 15, 14),
)


def _run(x, dw, w1, w2, grn_g, grn_b, cfg):
    B, H, W, C = x.shape
    F = w1.shape[1]
    assert B == 1 and dw.shape[:2] == (1, 1)
    N = H * W
    TM = cfg["TM"]
    T = N // TM
    assert N % TM == 0 and T % cfg["U1"] == 0 and cfg["NX"] > 2 * cfg["U1"] and cfg["NS"] >= 2 * cfg["U1"]
    cfg = dict(cfg, T=T)
    n_spilled = T - cfg["NCACHE"] - cfg["NS"]
    hbm, vmem = pl.BlockSpec(memory_space=pl.ANY), pl.BlockSpec(memory_space=pltpu.VMEM)
    out, _ = pl.pallas_call(
        functools.partial(_kernel, cfg=cfg),
        in_specs=[hbm, vmem, hbm, hbm, vmem, vmem],
        out_specs=[hbm, hbm],
        out_shape=[
            jax.ShapeDtypeStruct((N, C), x.dtype),
            jax.ShapeDtypeStruct((n_spilled, F // 128, TM, 128), jnp.bfloat16),
        ],
        scratch_shapes=[
            pltpu.VMEM((cfg["NX"], TM + 16, C), x.dtype),
            pltpu.VMEM((cfg["NS"] + cfg["NCACHE"], F // 128, TM, 128), jnp.bfloat16),
            pltpu.VMEM((15, C // 6, F // 3), jnp.uint32),
            pltpu.VMEM((cfg["AHEAD"], 15, cfg["R1"], C // 3), jnp.bfloat16),
            pltpu.VMEM((8, F), jnp.float32),
            pltpu.SemaphoreType.DMA((cfg["NX"],)),
            pltpu.SemaphoreType.DMA((cfg["NX"],)),
            pltpu.SemaphoreType.DMA((cfg["NS"],)),
        ],
        compiler_params=pltpu.CompilerParams(
            vmem_limit_bytes=int(cfg["VMEM_MB"] * 1024 * 1024), flags=cfg.get("FLAGS"),
            disable_bounds_checks=bool(cfg.get("NOBC"))),
    )(
        x.reshape(N, C),
        dw.reshape(1, C),
        w1.astype(jnp.bfloat16),
        w2.astype(jnp.bfloat16),
        grn_g.reshape(1, F),
        grn_b.reshape(1, F).astype(jnp.bfloat16),
    )
    return out.reshape(B, H, W, C)


@jax.jit
def pallas_standalone__modern_conv_block_slak__vision_kernel(
    x: jax.Array,
    dw: jax.Array,
    w1: jax.Array,
    w2: jax.Array,
    grn_g: jax.Array,
    grn_b: jax.Array,
):
    return _run(x, dw, w1, w2, grn_g, grn_b, _DEFAULT_CFG)
```

```python
import functools
import math

import jax
import jax.numpy as jnp
import jax.experimental.pallas as pl
import jax.experimental.pallas.tpu as pltpu

_LN_EPS = 1e-5
_GRN_EPS = 1e-6
_C0 = math.sqrt(2.0 / math.pi)
_BETA = (0.044715 * _C0) ** (1.0 / 3.0)
_KAPPA = _C0 / _BETA
_HSCALE = 1.0 / (2.0 * _BETA)

_HK = dict(
    sums={"s1": ("a00", -1, "a10"), "s6": ("a02", -1, "a12"), "s7": ("a00", 1, "a01"), "s8": ("s1", 1, "a01"),
          "s9": ("s8", -1, "a11"), "s10": ("a11", 1, "a12"), "s11": ("a11", -1, "s6"), "s12": ("s11", -1, "a01"),
          "s13": ("a10", 1, "a02"), "s14": ("a10", 1, "a12"), "s15": ("a00", 1, "a02")},
    left={1: "s1", 2: "a10", 3: "a01", 4: "a11", 5: "a02", 6: "s6", 7: "s7", 8: "s8", 9: "s9", 10: "s10",
          11: "s11", 12: "s12", 13: "s13", 14: "s14", 15: "s15"},
    right={
        1: {(0, 0): 1, (0, 2): -1, (1, 0): -1},
        2: {(0, 0): 1, (0, 1): -1, (2, 0): -1},
        3: {(1, 1): 1, (0, 1): -1, (1, 2): -1},
        4: {(1, 1): 1, (1, 0): -1, (2, 1): -1},
        5: {(2, 2): 1, (0, 2): -1, (2, 1): -1},
        6: {(1, 2): 1, (2, 0): 1, (2, 2): -1},
        7: {(0, 1): 1},
        8: {(1, 0): 1, (0, 1): -1},
        9: {(1, 0): -1},
        10: {(2, 1): 1},
        11: {(1, 2): 1, (2, 1): -1},
        12: {(1, 2): -1},
        13: {(2, 0): 1, (0, 2): -1},
        14: {(2, 0): 1},
        15: {(0, 2): 1},
    },
    shared={"q8": ("m7", 1, "m8"), "q9": ("q8", 1, "m9"), "q11": ("m10", 1, "m11"), "q12": ("q11", 1, "m12")},
    outputs={
        (0, 0): {"m1": 1, "m2": 1, "q8": 1, "m13": 1, "m15": 1},
        (0, 1): {"m3": 1, "m7": 1, "q12": 1},
        (0, 2): {"m5": 1, "q12": 1, "m15": 1},
        (1, 0): {"m2": 1, "q9": 1, "m14": 1},
        (1, 1): {"m4": 1, "q9": 1, "m10": 1},
        (1, 2): {"m5": 1, "m6": 1, "q11": 1, "m13": -1, "m14": 1},
    },
)


def _left_operands(scheme, a):
    vals = {"a%d%d" % (i, p): a[i][p] for i in range(2) for p in range(3)}
    for name, (u, sign, v) in scheme["sums"].items():
        vals[name] = vals[u] + vals[v] if sign > 0 else vals[u] - vals[v]
    return {r: vals[name] for r, name in scheme["left"].items()}


def _right_operand(scheme, r, block):
    pos = [block(*pq) for pq, sign in scheme["right"][r].items() if sign > 0]
    neg = [block(*pq) for pq, sign in scheme["right"][r].items() if sign < 0]
    total = functools.reduce(lambda u, v: u + v, pos) if pos else -neg.pop()
    return functools.reduce(lambda u, v: u - v, neg, total)


class _BlockProduct:
    def __init__(self, scheme, product, emit, eager=False):
        self.shared, self.product, self.emit, self.eager = dict(scheme["shared"]), product, emit, eager
        self.ready, self.partial = {}, {}
        self.missing = {iq: dict(terms) for iq, terms in scheme["outputs"].items()}

    def _fold(self, iq, name):
        sign, value = self.missing[iq].pop(name), self.ready[name]
        if iq in self.partial:
            have, total = self.partial[iq]
            if have == sign:
                value = total + value
            else:
                sign, value = 1, (total - value if have > 0 else value - total)
        self.partial[iq] = (sign, value)

    def step(self, r):
        fresh = ["m%d" % r]
        self.ready[fresh[0]] = self.product(r)
        for name, (u, sign, v) in list(self.shared.items()):
            if u in self.ready and v in self.ready:
                self.ready[name] = self.ready[u] + self.ready[v] if sign > 0 else self.ready[u] - self.ready[v]
                fresh.append(name)
                del self.shared[name]
        for iq, terms in list(self.missing.items()):
            if all(name in self.ready for name in terms):
                for name in [n for n in self.ready if n in terms]:
                    self._fold(iq, name)
                self.emit(*iq, self.partial[iq][1])
                del self.missing[iq]
        for name in fresh:
            users = [iq for iq, terms in self.missing.items() if name in terms]
            pending = any(name in (u, v) for u, _, v in self.shared.values())
            if self.eager or (len(users) == 1 and not pending):
                for iq in users:
                    self._fold(iq, name)


def _pack(v):
    return pltpu.bitcast(v.astype(jnp.bfloat16), jnp.uint32)


def _unpack(v):
    return pltpu.bitcast(v, jnp.bfloat16)


def _kernel(x_hbm, dw_ref, w1_hbm, w2_hbm, g_ref, b_ref, o_hbm, h_hbm,
            xbuf, hbuf, wc, lhs0, acc, xsem, osem, hsem, *, cfg):
    TM, T, NCACHE, NS, NX = (cfg[k] for k in ("TM", "T", "NCACHE", "NS", "NX"))
    R1, R2, U1 = cfg["R1"], cfg["R2"], cfg["U1"]
    F, C = w2_hbm.shape
    CB, FB = C // 3, F // 3
    NSPILL = T - NCACHE - NS
    f32, bf16 = jnp.float32, jnp.bfloat16
    sch1 = sch2 = _HK
    products = range(1, 16)

    def place(t):
        span = T - cfg["TAIL"]
        before = jnp.minimum(t * NCACHE // span, NCACHE)
        ring = jnp.minimum((t + 1) * NCACHE // span, NCACHE) == before
        s = t - before
        return ring, s, jnp.where(ring, s % NS, NS + before)

    def x_load(t):
        return pltpu.make_async_copy(x_hbm.at[pl.ds(t * TM, TM)], xbuf.at[t % NX, pl.ds(0, TM)], xsem.at[t % NX])

    NW = pl.cdiv(F, TM)

    def w2_load(k):
        n, slot = min(TM, F - k * TM), (T + k) % NX
        return pltpu.make_async_copy(w2_hbm.at[pl.ds(k * TM, n)], xbuf.at[slot, pl.ds(0, n)], xsem.at[slot])

    def w2_tile(r0, c0):
        return xbuf[(T + r0 // TM) % NX, r0 % TM:r0 % TM + CB, c0:c0 + CB]

    def o_store(t):
        return pltpu.make_async_copy(xbuf.at[t % NX, pl.ds(0, TM)], o_hbm.at[pl.ds(t * TM, TM)], osem.at[t % NX])

    def h_store(s):
        return pltpu.make_async_copy(hbuf.at[s % NS], h_hbm.at[s], hsem.at[s % NS])

    def h_load(s):
        return pltpu.make_async_copy(h_hbm.at[s], hbuf.at[s % NS], hsem.at[s % NS])

    w1_loads = [pltpu.make_async_copy(w1_hbm.at[:, pl.ds(j * CB, CB)], hbuf.at[NS + NCACHE - 1, j, pl.ds(0, C)],
                                      hsem.at[0]) for j in range(F // CB)]
    x_load(0).start()
    for load in w1_loads:
        load.start()

    def h_block(slot, r0, n, p):
        return jnp.concatenate([hbuf[slot, p * (FB // CB) + k, r0:r0 + n, :].astype(f32)
                                for k in range(FB // CB)], axis=1)

    for t in range(1, U1 + 1):
        x_load(t).start()
    acc[...] = jnp.zeros_like(acc)
    dw = dw_ref[...].astype(f32)

    def layernorm(xs, r0, n):
        y = xbuf[xs, r0:r0 + n, :].astype(f32) * dw
        d = y - jnp.sum(y, axis=-1, keepdims=True) * (1.0 / C)
        v = jnp.sum(d * d, axis=-1, keepdims=True) + C * _LN_EPS
        return d * jnp.exp2(-0.5 * jnp.log2(v))

    def operands1(rows):
        a = [[u[:, p * CB:(p + 1) * CB] for p in range(3)] for u in rows]
        return {r: v.astype(bf16) for r, v in _left_operands(sch1, a).items()}

    x_load(0).wait()
    AHEAD = cfg["AHEAD"]
    for sub in range(AHEAD):
        for r, v in operands1([layernorm(0, (2 * sub + i) * R1, R1) for i in range(2)]).items():
            lhs0[sub, r - 1] = v
    for load in w1_loads:
        load.wait()
    for r in products[:cfg.get("NPREP")]:
        wc[r - 1] = _pack((_BETA * math.sqrt(C)) * _right_operand(
            sch1, r, lambda p, q: h_block(NS + NCACHE - 1, p * CB, CB, q)))

    def places(t0, step, n):
        return [place(t0 + step * u) for u in range(n)]

    def sweep1(it, carry):
        t0 = it * U1
        done, tiles = carry
        for ring, s, _ in tiles:
            @pl.when(jnp.logical_and(ring, s >= NS))
            def _():
                h_store(s - NS).wait()
        for u in range(1, U1):
            x_load(t0 + u).wait()

        @pl.when(t0 + U1 < T)
        def _():
            x_load(t0 + U1).wait()

        @pl.when(t0 + U1 == T)
        def _():
            w2_load(0).wait()

        def start_copies():
            for ring, s, _ in done:
                @pl.when(jnp.logical_and(ring, s < NSPILL))
                def _():
                    h_store(s).start()
            for u in range(U1):
                @pl.when(t0 + U1 + 1 + u < T)
                def _():
                    x_load(t0 + U1 + 1 + u).start()
            for k in range(NW):
                @pl.when(it == (T + k - U1 - 1) // U1)
                def _():
                    w2_load(k).start()

        per_tile = TM // (2 * R1)
        nsub = U1 * per_tile
        nstream = len(cfg["LAG"])
        SW = FB // nstream
        sumsq = {}

        latest = []

        def product(lhs, c, r):
            latest[:] = [jnp.dot(lhs[r], _unpack(wc[r - 1, :, c * SW:(c + 1) * SW]), preferred_element_type=f32)]
            return latest[0]

        def emit(sub, c, i, q, w):
            h = w * jnp.tanh(w * (w * w + _KAPPA)) + w
            r0, c0 = (sub % per_tile * 2 + i) * R1, q * FB + c * SW
            for k in range(SW // CB):
                hbuf[tiles[sub // per_tile][2], c0 // CB + k, r0:r0 + R1, :] = h[:, k * CB:(k + 1) * CB].astype(bf16)
            sq = jnp.sum((h * h).reshape(R1 // 8, 8, SW), axis=0)
            sumsq[c0] = sumsq[c0] + sq if c0 in sumsq else sq

        operands = {sub: {r: lhs0[sub, r - 1] for r in products} for sub in range(AHEAD)}

        gates = cfg["GATES"]
        PR = 2 * R1 // len(gates)

        def norm_piece(sub, k, gated):
            if gated:
                xbuf[(t0 + U1 + 1) % NX, TM:TM + 8, 0:CB] = latest[0][0:8, 0:CB].astype(xbuf.dtype)
            r0 = sub % per_tile * 2 * R1 + k % 2 * R1 + k // 2 * PR
            return layernorm((t0 + sub // per_tile) % NX, r0, PR)

        def stream(c):
            prev = None
            for sub in range(nsub + 1):
                if sub < nsub:
                    cur = _BlockProduct(sch1, functools.partial(product, operands[sub], c),
                                        functools.partial(emit, sub, c), cfg['EAGER1'])
                pieces = {}
                for n, r in enumerate(cfg["ORDER1"][c]):
                    if r > 0 and sub < nsub:
                        cur.step(r)
                    elif r < 0 and prev is not None:
                        prev.step(-r)
                    if c == 0 and sub < nsub:
                        for k, gate in enumerate(gates):
                            if sub == nsub - 1:
                                gate = min(gate, cfg.get("LASTGATE", -1))
                            if max(gate, 0) == n:
                                pieces[k] = norm_piece(sub + AHEAD, k, gate >= 0)
                    if (r > 0 and sub < nsub) or (r < 0 and prev is not None):
                        yield
                if c == 0 and sub < nsub:
                    operands[sub + AHEAD] = operands1(
                        [jnp.concatenate([pieces[k] for k in range(i, len(gates), 2)], axis=0) for i in range(2)])
                prev = cur

        streams = [stream(c) for c in range(nstream)]
        for n in range(15 * nsub + max(cfg["LAG"])):
            for c, lag in enumerate(cfg["LAG"]):
                if 0 <= n - lag < 15 * nsub:
                    next(streams[c])
            if n == cfg["START1"]:
                start_copies()
        for rest in streams:
            next(rest, None)
        for c0, v in sumsq.items():
            acc[:, c0:c0 + SW] += v
        for sub in range(AHEAD):
            for r, v in operands[nsub + sub].items():
                lhs0[sub, r - 1] = v
        return tiles, places(t0 + U1, 1, U1)

    first = places(jnp.int32(0), 1, U1)
    nothing = [(jnp.logical_and(ring, False), s, slot) for ring, s, slot in first]
    jax.lax.fori_loop(0, T // U1, sweep1, (nothing, first))

    gx = jnp.sqrt(jnp.sum(acc[...], axis=0, keepdims=True) * _HSCALE ** 2 + _GRN_EPS)
    nx = gx / (jnp.sum(gx, axis=-1, keepdims=True) * (1.0 / F) + _GRN_EPS)
    scale = (g_ref[...].astype(f32).reshape(1, F) * nx + 1.0) * _HSCALE
    for k in range(1, NW):
        w2_load(k).wait()
    for k in range(FB // CB):
        rows = [p * FB + k * CB for p in range(3)]
        col = [jnp.transpose(jnp.broadcast_to(scale[:, r0:r0 + CB], (CB, CB))) for r0 in rows]
        scaled = [[w2_tile(rows[p], q * CB).astype(f32) * col[p] for q in range(3)] for p in range(3)]
        for r in products:
            wc[r - 1, :, k * CB:(k + 1) * CB] = _pack(_right_operand(sch2, r, lambda p, q: scaled[p][q]))
    w2 = jnp.concatenate([jnp.concatenate([w2_tile(r0, c0) for c0 in range(0, C, CB)], axis=1)
                          for r0 in range(0, F, CB)], axis=0)
    bias = jnp.dot(jnp.broadcast_to(b_ref[...].astype(f32).reshape(1, F), (16, F)).astype(bf16), w2, preferred_element_type=f32)[0:1, :]
    for k in reversed(range(NW)):
        x_load(T - NX + k).start()

    SLACK = cfg["SLACK"]

    def compute(t, slot, hook):
        xs = t % NX
        for sub in range(TM // (2 * R2)):
            r0 = sub * 2 * R2
            ops = _left_operands(sch2, [
                [h_block(slot, r0 + i * R2, R2, p) for p in range(3)] for i in range(2)])

            def product(r):
                w = jnp.concatenate(
                    [_unpack(wc[r - 1, :, k * CB:(k + 1) * CB]) for k in range(FB // CB)], axis=0)
                return jnp.dot(ops[r].astype(bf16), w, preferred_element_type=f32)

            def emit(i, q, y):
                rows, cols = slice(r0 + i * R2, r0 + (i + 1) * R2), slice(q * CB, (q + 1) * CB)
                xbuf[xs, rows, cols] = (y + bias[:, cols] + xbuf[xs, rows, cols].astype(f32)).astype(xbuf.dtype)

            bp = _BlockProduct(sch2, product, emit, cfg['EAGER2'])
            for n, r in enumerate(cfg["ORDER2"]):
                bp.step(r)
                if (sub, n) == cfg["HOOK"]:
                    hook()

    def sweep2(step, carry):
        t = T - 1 - step
        (done_ring, done_s, _), (ring, s, slot) = carry

        def release():
            @pl.when(jnp.logical_and(done_ring, done_s >= NS))
            def _():
                h_load(done_s - NS).start()

            @pl.when(step > 0)
            def _():
                o_store(t + 1).start()

        if cfg["EARLY"]:
            release()

        @pl.when(t + SLACK < T)
        def _():
            o_store(t + SLACK).wait()

        def refill():
            @pl.when(jnp.logical_and(t + SLACK < T, t + SLACK >= NX))
            def _():
                x_load(t + SLACK - NX).start()

        if cfg["EARLY"] > 1:
            refill()

        @pl.when(jnp.logical_and(ring, s < NSPILL))
        def _():
            h_load(s).wait()

        @pl.when(t < T - NX + NW)
        def _():
            x_load(t).wait()

        def start_copies():
            if not cfg["EARLY"]:
                release()
            if cfg["EARLY"] < 2:
                refill()

        compute(t, slot, start_copies)
        return (ring, s, slot), place(jnp.maximum(t - 1, 0))

    last = place(jnp.int32(T - 1))
    jax.lax.fori_loop(0, T, sweep2, ((jnp.logical_and(last[0], False), *last[1:]), last))
    o_store(0).start()
    for t in range(SLACK):
        o_store(t).wait()


_DEFAULT_CFG = dict(
    TM=1024, NCACHE=36, NS=4, TAIL=4, NX=5, SLACK=2, U1=2, U2=1, R1=32, R2=64, VMEM_MB=127.9,
    ORDER1=((8, 9, 7, 4, 2, 14, 10, 6, 13, 11, 12, 3, 5, 15, 1),) * 2 + ((8, 7, 2, 9, 10, 4, 14, 6, 13, 11, 12, 3, 5, 15, 1),) * 2,
    LAG=(0, 0, 10, 11), GATES=(1, 2, 4, 5, 6, 8, 10, 11), AHEAD=2,
    EAGER1=1, EAGER2=1, HOOK=(0, 1), START1=2, EARLY=0, NOBC=1,
    ORDER2=(5, 2, 1, 8, 9, 7, 4, 3, 6, 11, 10, 13, 12, 15, 14),
)


def _run(x, dw, w1, w2, grn_g, grn_b, cfg):
    B, H, W, C = x.shape
    F = w1.shape[1]
    assert B == 1 and dw.shape[:2] == (1, 1)
    N = H * W
    TM = cfg["TM"]
    T = N // TM
    assert N % TM == 0 and T % cfg["U1"] == 0 and cfg["NX"] > 2 * cfg["U1"] and cfg["NS"] >= 2 * cfg["U1"]
    cfg = dict(cfg, T=T)
    n_spilled = T - cfg["NCACHE"] - cfg["NS"]
    hbm, vmem = pl.BlockSpec(memory_space=pl.ANY), pl.BlockSpec(memory_space=pltpu.VMEM)
    out, _ = pl.pallas_call(
        functools.partial(_kernel, cfg=cfg),
        in_specs=[hbm, vmem, hbm, hbm, vmem, vmem],
        out_specs=[hbm, hbm],
        out_shape=[
            jax.ShapeDtypeStruct((N, C), x.dtype),
            jax.ShapeDtypeStruct((n_spilled, F // 128, TM, 128), jnp.bfloat16),
        ],
        scratch_shapes=[
            pltpu.VMEM((cfg["NX"], TM + 16, C), x.dtype),
            pltpu.VMEM((cfg["NS"] + cfg["NCACHE"], F // 128, TM, 128), jnp.bfloat16),
            pltpu.VMEM((15, C // 6, F // 3), jnp.uint32),
            pltpu.VMEM((cfg["AHEAD"], 15, cfg["R1"], C // 3), jnp.bfloat16),
            pltpu.VMEM((8, F), jnp.float32),
            pltpu.SemaphoreType.DMA((cfg["NX"],)),
            pltpu.SemaphoreType.DMA((cfg["NX"],)),
            pltpu.SemaphoreType.DMA((cfg["NS"],)),
        ],
        compiler_params=pltpu.CompilerParams(
            vmem_limit_bytes=int(cfg["VMEM_MB"] * 1024 * 1024), flags=cfg.get("FLAGS"),
            disable_bounds_checks=bool(cfg.get("NOBC"))),
    )(
        x.reshape(N, C),
        dw.reshape(1, C),
        w1.astype(jnp.bfloat16),
        w2.astype(jnp.bfloat16),
        grn_g,
        grn_b,
    )
    return out.reshape(B, H, W, C)


@jax.jit
def pallas_standalone__modern_conv_block_slak__vision_kernel(
    x: jax.Array,
    dw: jax.Array,
    w1: jax.Array,
    w2: jax.Array,
    grn_g: jax.Array,
    grn_b: jax.Array,
):
    return _run(x, dw, w1, w2, grn_g, grn_b, _DEFAULT_CFG)
```

```python
import functools
import math

import jax
import jax.numpy as jnp
import jax.experimental.pallas as pl
import jax.experimental.pallas.tpu as pltpu

_LN_EPS = 1e-5
_GRN_EPS = 1e-6
_C0 = math.sqrt(2.0 / math.pi)
_BETA = (0.044715 * _C0) ** (1.0 / 3.0)
_KAPPA = _C0 / _BETA
_HSCALE = 1.0 / (2.0 * _BETA)

_PRODUCTS = tuple(range(1, 16))
_RIGHT = {
    1: {(0, 0): 1, (0, 2): -1, (1, 0): -1},
    2: {(0, 0): 1, (0, 1): -1, (2, 0): -1},
    3: {(1, 1): 1, (0, 1): -1, (1, 2): -1},
    4: {(1, 1): 1, (1, 0): -1, (2, 1): -1},
    5: {(2, 2): 1, (0, 2): -1, (2, 1): -1},
    6: {(1, 2): 1, (2, 0): 1, (2, 2): -1},
    7: {(0, 1): 1},
    8: {(1, 0): 1, (0, 1): -1},
    9: {(1, 0): -1},
    10: {(2, 1): 1},
    11: {(1, 2): 1, (2, 1): -1},
    12: {(1, 2): -1},
    13: {(2, 0): 1, (0, 2): -1},
    14: {(2, 0): 1},
    15: {(0, 2): 1},
}
_SHARED = {"q8": ("m7", "m8"), "q9": ("q8", "m9"), "q11": ("m10", "m11"), "q12": ("q11", "m12")}
_OUTPUTS = {
    (0, 0): {"m1": 1, "m2": 1, "q8": 1, "m13": 1, "m15": 1},
    (0, 1): {"m3": 1, "m7": 1, "q12": 1},
    (0, 2): {"m5": 1, "q12": 1, "m15": 1},
    (1, 0): {"m2": 1, "q9": 1, "m14": 1},
    (1, 1): {"m4": 1, "q9": 1, "m10": 1},
    (1, 2): {"m5": 1, "m6": 1, "q11": 1, "m13": -1, "m14": 1},
}


def _left_operands(a):
    (a00, a01, a02), (a10, a11, a12) = a
    s1, s6 = a00 - a10, a02 - a12
    s7, s8 = a00 + a01, s1 + a01
    s9, s10, s11 = s8 - a11, a11 + a12, a11 - s6
    s12, s13, s14, s15 = s11 - a01, a10 + a02, a10 + a12, a00 + a02
    ops = (s1, a10, a01, a11, a02, s6, s7, s8, s9, s10, s11, s12, s13, s14, s15)
    return {r: v.astype(jnp.bfloat16) for r, v in zip(_PRODUCTS, ops)}


def _right_operand(r, block):
    pos = [block(*pq) for pq, sign in _RIGHT[r].items() if sign > 0]
    neg = [block(*pq) for pq, sign in _RIGHT[r].items() if sign < 0]
    total = functools.reduce(lambda u, v: u + v, pos) if pos else -neg.pop()
    return functools.reduce(lambda u, v: u - v, neg, total)


class _BlockProduct:
    def __init__(self, emit):
        self.emit = emit
        self.ready, self.partial = {}, {}
        self.missing = {iq: dict(terms) for iq, terms in _OUTPUTS.items()}

    def add(self, r, product):
        fresh = ["m%d" % r]
        self.ready[fresh[0]] = product
        for name, (u, v) in _SHARED.items():
            if name not in self.ready and u in self.ready and v in self.ready:
                self.ready[name] = self.ready[u] + self.ready[v]
                fresh.append(name)
        complete = [iq for iq, terms in self.missing.items() if all(name in self.ready for name in terms)]
        for iq in complete:
            self._fold(iq, fresh)
            self.emit(*iq, self.partial[iq][1])
            del self.missing[iq]
        for name in fresh:
            for iq in self.missing:
                self._fold(iq, [name])

    def _fold(self, iq, names):
        for name in names:
            if name not in self.missing[iq]:
                continue
            sign, value = self.missing[iq].pop(name), self.ready[name]
            if iq in self.partial:
                have, total = self.partial[iq]
                if have == sign:
                    value = total + value
                else:
                    sign, value = 1, (total - value if have > 0 else value - total)
            self.partial[iq] = (sign, value)


def _pack(v):
    return pltpu.bitcast(v.astype(jnp.bfloat16), jnp.uint32)


def _unpack(v):
    return pltpu.bitcast(v, jnp.bfloat16)


def _kernel(x_hbm, dw_ref, w1_hbm, w2_hbm, g_ref, b_ref, o_hbm, h_hbm,
            xbuf, hbuf, wc, lhs0, acc, xsem, osem, hsem, *, cfg):
    TM, NCACHE, NS, NX, U = (cfg[k] for k in ("TM", "NCACHE", "NS", "NX", "U"))
    R1, R2, AHEAD, SLACK = (cfg[k] for k in ("R1", "R2", "AHEAD", "SLACK"))
    F, C = w2_hbm.shape
    CB, FB = C // 3, F // 3
    T = x_hbm.shape[0] // TM
    NSPILL = T - NCACHE - NS
    NW = pl.cdiv(F, TM)
    f32, bf16 = jnp.float32, jnp.bfloat16

    def place(t):
        span = T - NS
        before = jnp.minimum(t * NCACHE // span, NCACHE)
        ring = jnp.minimum((t + 1) * NCACHE // span, NCACHE) == before
        s = t - before
        return ring, s, jnp.where(ring, s % NS, NS + before)

    def nowhere(placed):
        return (jnp.logical_and(placed[0], False), *placed[1:])

    def x_load(t):
        return pltpu.make_async_copy(x_hbm.at[pl.ds(t * TM, TM)], xbuf.at[t % NX, pl.ds(0, TM)], xsem.at[t % NX])

    def o_store(t):
        return pltpu.make_async_copy(xbuf.at[t % NX, pl.ds(0, TM)], o_hbm.at[pl.ds(t * TM, TM)], osem.at[t % NX])

    def h_store(s):
        return pltpu.make_async_copy(hbuf.at[s % NS], h_hbm.at[s], hsem.at[s % NS])

    def h_load(s):
        return pltpu.make_async_copy(h_hbm.at[s], hbuf.at[s % NS], hsem.at[s % NS])

    def w2_load(k):
        n, slot = min(TM, F - k * TM), (T + k) % NX
        return pltpu.make_async_copy(w2_hbm.at[pl.ds(k * TM, n)], xbuf.at[slot, pl.ds(0, n)], xsem.at[slot])

    def w2_tile(r0, c0):
        return xbuf[(T + r0 // TM) % NX, r0 % TM:r0 % TM + CB, c0:c0 + CB]

    def h_block(slot, r0, n, p):
        return jnp.concatenate(
            [hbuf[slot, p * (FB // CB) + k, r0:r0 + n, :].astype(f32) for k in range(FB // CB)], axis=1)

    def layernorm(t, r0, n):
        y = xbuf[t % NX, r0:r0 + n, :].astype(f32) * dw
        d = y - jnp.sum(y, axis=-1, keepdims=True) * (1.0 / C)
        v = jnp.sum(d * d, axis=-1, keepdims=True) + C * _LN_EPS
        return d * jnp.exp2(-0.5 * jnp.log2(v))

    def operands1(rows):
        return _left_operands([[u[:, p * CB:(p + 1) * CB] for p in range(3)] for u in rows])

    staging = NS + NCACHE - 1
    w1_loads = [pltpu.make_async_copy(w1_hbm.at[:, pl.ds(j * CB, CB)], hbuf.at[staging, j, pl.ds(0, C)], hsem.at[0])
                for j in range(F // CB)]
    x_load(0).start()
    for load in w1_loads:
        load.start()
    for t in range(1, U + 1):
        x_load(t).start()
    acc[...] = jnp.zeros_like(acc)
    dw = dw_ref[...].astype(f32)
    x_load(0).wait()
    for sub in range(AHEAD):
        for r, v in operands1([layernorm(0, (2 * sub + i) * R1, R1) for i in range(2)]).items():
            lhs0[sub, r - 1] = v
    for load in w1_loads:
        load.wait()
    for r in _PRODUCTS:
        wc[r - 1] = _pack((_BETA * math.sqrt(C)) * _right_operand(r, lambda p, q: h_block(staging, p * CB, CB, q)))

    def sweep1(it, carry):
        t0 = it * U
        done, tiles = carry
        for ring, s, _ in tiles:
            @pl.when(jnp.logical_and(ring, s >= NS))
            def _():
                h_store(s - NS).wait()
        for u in range(1, U):
            x_load(t0 + u).wait()

        @pl.when(t0 + U < T)
        def _():
            x_load(t0 + U).wait()

        @pl.when(t0 + U == T)
        def _():
            w2_load(0).wait()

        def start_copies():
            for ring, s, _ in done:
                @pl.when(jnp.logical_and(ring, s < NSPILL))
                def _():
                    h_store(s).start()
            for t in [t0 + U + 1 + u for u in range(U)]:
                @pl.when(t < T)
                def _():
                    x_load(t).start()
            for k in range(NW):
                @pl.when(it == (T + k - U - 1) // U)
                def _():
                    w2_load(k).start()

        per_tile = TM // (2 * R1)
        nsub = U * per_tile
        sumsq = {}
        operands = {sub: {r: lhs0[sub, r - 1] for r in _PRODUCTS} for sub in range(AHEAD)}

        def emit(sub, c, i, q, w):
            h = w * jnp.tanh(w * (w * w + _KAPPA)) + w
            r0, j = (sub % per_tile * 2 + i) * R1, q * (FB // CB) + c
            hbuf[tiles[sub // per_tile][2], j, r0:r0 + R1, :] = h.astype(bf16)
            sq = jnp.sum((h * h).reshape(R1 // 8, 8, CB), axis=0)
            sumsq[j] = sumsq[j] + sq if j in sumsq else sq

        def stream(c):
            gates = cfg["GATES"]
            n_rows = 2 * R1 // len(gates)
            for sub in range(nsub):
                block_product = _BlockProduct(functools.partial(emit, sub, c))
                pieces = []
                for n, r in enumerate(cfg["ORDER1"][c]):
                    m = jnp.dot(operands[sub][r], _unpack(wc[r - 1, :, c * CB:(c + 1) * CB]),
                                preferred_element_type=f32)
                    block_product.add(r, m)
                    for k, gate in enumerate(gates if c == 0 else ()):
                        last = sub == nsub - 1
                        if n == (0 if last else gate):
                            if not last:
                                xbuf[(t0 + U + 1) % NX, TM:TM + 8, 0:CB] = m[0:8].astype(xbuf.dtype)
                            later = sub + AHEAD
                            r0 = later % per_tile * 2 * R1 + k % 2 * R1 + k // 2 * n_rows
                            pieces.append(layernorm(t0 + later // per_tile, r0, n_rows))
                    yield
                if c == 0:
                    operands[sub + AHEAD] = operands1([jnp.concatenate(pieces[i::2], axis=0) for i in range(2)])

        streams = [stream(c) for c in range(FB // CB)]
        for n in range(15 * nsub + max(cfg["LAG"])):
            for steps, lag in zip(streams, cfg["LAG"]):
                if 0 <= n - lag < 15 * nsub:
                    next(steps)
            if n == 2:
                start_copies()
        for steps in streams:
            next(steps, None)
        for j, v in sumsq.items():
            acc[:, j * CB:(j + 1) * CB] += v
        for sub in range(AHEAD):
            for r, v in operands[nsub + sub].items():
                lhs0[sub, r - 1] = v
        return tiles, [place(t0 + U + u) for u in range(U)]

    first = [place(jnp.int32(u)) for u in range(U)]
    jax.lax.fori_loop(0, T // U, sweep1, ([nowhere(p) for p in first], first))

    gx = jnp.sqrt(jnp.sum(acc[...], axis=0, keepdims=True) * _HSCALE ** 2 + _GRN_EPS)
    nx = gx / (jnp.sum(gx, axis=-1, keepdims=True) * (1.0 / F) + _GRN_EPS)
    scale = (g_ref[...].astype(f32).reshape(1, F) * nx + 1.0) * _HSCALE
    for k in range(1, NW):
        w2_load(k).wait()
    for k in range(FB // CB):
        rows = [p * FB + k * CB for p in range(3)]
        col = [jnp.transpose(jnp.broadcast_to(scale[:, r0:r0 + CB], (CB, CB))) for r0 in rows]
        scaled = [[w2_tile(rows[p], q * CB).astype(f32) * col[p] for q in range(3)] for p in range(3)]
        for r in _PRODUCTS:
            wc[r - 1, :, k * CB:(k + 1) * CB] = _pack(_right_operand(r, lambda p, q: scaled[p][q]))
    w2 = jnp.concatenate([jnp.concatenate([w2_tile(r0, c0) for c0 in range(0, C, CB)], axis=1)
                          for r0 in range(0, F, CB)], axis=0)
    b = jnp.broadcast_to(b_ref[...].astype(f32).reshape(1, F), (16, F)).astype(bf16)
    bias = jnp.dot(b, w2, preferred_element_type=f32)[0:1, :]
    for k in reversed(range(NW)):
        x_load(T - NX + k).start()

    def sweep2(step, carry):
        t = T - 1 - step
        (done_ring, done_s, _), (ring, s, slot) = carry

        @pl.when(t + SLACK < T)
        def _():
            o_store(t + SLACK).wait()

        @pl.when(jnp.logical_and(ring, s < NSPILL))
        def _():
            h_load(s).wait()

        @pl.when(t < T - NX + NW)
        def _():
            x_load(t).wait()

        @pl.when(step > 0)
        def _():
            o_store(t + 1).start()

        @pl.when(jnp.logical_and(t + SLACK < T, t + SLACK >= NX))
        def _():
            x_load(t + SLACK - NX).start()

        for r0 in range(0, TM, 2 * R2):
            if r0 == 2 * R2:
                @pl.when(jnp.logical_and(done_ring, done_s >= NS))
                def _():
                    h_load(done_s - NS).start()

            def emit(i, q, y):
                rows, cols = slice(r0 + i * R2, r0 + (i + 1) * R2), slice(q * CB, (q + 1) * CB)
                xbuf[t % NX, rows, cols] = (
                    y + bias[:, cols] + xbuf[t % NX, rows, cols].astype(f32)).astype(xbuf.dtype)

            ops = _left_operands([[h_block(slot, r0 + i * R2, R2, p) for p in range(3)] for i in range(2)])
            block_product = _BlockProduct(emit)
            for r in cfg["ORDER2"]:
                w = jnp.concatenate(
                    [_unpack(wc[r - 1, :, k * CB:(k + 1) * CB]) for k in range(FB // CB)], axis=0)
                block_product.add(r, jnp.dot(ops[r], w, preferred_element_type=f32))
        return (ring, s, slot), place(jnp.maximum(t - 1, 0))

    last = place(jnp.int32(T - 1))
    jax.lax.fori_loop(0, T, sweep2, (nowhere(last), last))
    o_store(0).start()
    for t in range(SLACK):
        o_store(t).wait()


_DEFAULT_CFG = dict(
    TM=1024,
    NCACHE=36, NS=4,
    NX=6, SLACK=2,
    U=2,
    R1=32, R2=64,
    ORDER1=((8, 9, 7, 4, 2, 14, 10, 6, 13, 11, 12, 3, 5, 15, 1), (9, 8, 7, 4, 2, 14, 10, 6, 13, 11, 12, 3, 5, 15, 1),
            (8, 7, 2, 9, 10, 4, 14, 6, 13, 11, 12, 3, 5, 15, 1), (8, 7, 2, 9, 4, 14, 10, 6, 13, 11, 12, 3, 5, 15, 1)),
    LAG=(0, 0, 10, 11), GATES=(1, 2, 4, 5, 6, 8, 10, 11), AHEAD=2,
    ORDER2=(5, 2, 1, 8, 9, 7, 4, 3, 6, 11, 10, 13, 12, 15, 14),
)


def _run(x, dw, w1, w2, grn_g, grn_b, cfg):
    B, H, W, C = x.shape
    F = w1.shape[1]
    N, TM = H * W, cfg["TM"]
    assert B == 1 and dw.shape == (1, 1, C) and C == 3 * 128 and F == 4 * C and x.dtype == jnp.bfloat16
    assert N % (TM * cfg["U"]) == 0 and cfg["NX"] > 2 * cfg["U"] and cfg["NS"] >= 2 * cfg["U"] and cfg["SLACK"] >= 2
    n_spilled = N // TM - cfg["NCACHE"] - cfg["NS"]
    hbm, vmem = pl.BlockSpec(memory_space=pl.ANY), pl.BlockSpec(memory_space=pltpu.VMEM)
    out, _ = pl.pallas_call(
        functools.partial(_kernel, cfg=cfg),
        in_specs=[hbm, vmem, hbm, hbm, vmem, vmem],
        out_specs=[hbm, hbm],
        out_shape=[
            jax.ShapeDtypeStruct((N, C), x.dtype),
            jax.ShapeDtypeStruct((n_spilled, F // 128, TM, 128), jnp.bfloat16),
        ],
        scratch_shapes=[
            pltpu.VMEM((cfg["NX"], TM + 16, C), x.dtype),
            pltpu.VMEM((cfg["NS"] + cfg["NCACHE"], F // 128, TM, 128), jnp.bfloat16),
            pltpu.VMEM((15, C // 6, F // 3), jnp.uint32),
            pltpu.VMEM((cfg["AHEAD"], 15, cfg["R1"], C // 3), jnp.bfloat16),
            pltpu.VMEM((8, F), jnp.float32),
            pltpu.SemaphoreType.DMA((cfg["NX"],)),
            pltpu.SemaphoreType.DMA((cfg["NX"],)),
            pltpu.SemaphoreType.DMA((cfg["NS"],)),
        ],
        compiler_params=pltpu.CompilerParams(vmem_limit_bytes=int(127.9 * 2 ** 20), disable_bounds_checks=True),
    )(x.reshape(N, C), dw.reshape(1, C), w1.astype(jnp.bfloat16), w2.astype(jnp.bfloat16), grn_g, grn_b)
    return out.reshape(B, H, W, C)


@jax.jit
def pallas_standalone__modern_conv_block_slak__vision_kernel(
    x: jax.Array,
    dw: jax.Array,
    w1: jax.Array,
    w2: jax.Array,
    grn_g: jax.Array,
    grn_b: jax.Array,
):
    return _run(x, dw, w1, w2, grn_g, grn_b, _DEFAULT_CFG)
```

```python
import functools
import math

import jax
import jax.numpy as jnp
import jax.experimental.pallas as pl
import jax.experimental.pallas.tpu as pltpu

_LN_EPS = 1e-5
_GRN_EPS = 1e-6
_C0 = math.sqrt(2.0 / math.pi)
_BETA = (0.044715 * _C0) ** (1.0 / 3.0)
_KAPPA = _C0 / _BETA
_HSCALE = 1.0 / (2.0 * _BETA)

_PRODUCTS = tuple(range(1, 16))
_RIGHT = {
    1: {(0, 0): 1, (0, 2): -1, (1, 0): -1},
    2: {(0, 0): 1, (0, 1): -1, (2, 0): -1},
    3: {(1, 1): 1, (0, 1): -1, (1, 2): -1},
    4: {(1, 1): 1, (1, 0): -1, (2, 1): -1},
    5: {(2, 2): 1, (0, 2): -1, (2, 1): -1},
    6: {(1, 2): 1, (2, 0): 1, (2, 2): -1},
    7: {(0, 1): 1},
    8: {(1, 0): 1, (0, 1): -1},
    9: {(1, 0): -1},
    10: {(2, 1): 1},
    11: {(1, 2): 1, (2, 1): -1},
    12: {(1, 2): -1},
    13: {(2, 0): 1, (0, 2): -1},
    14: {(2, 0): 1},
    15: {(0, 2): 1},
}
_SHARED = {"q8": ("m7", "m8"), "q9": ("q8", "m9"), "q11": ("m10", "m11"), "q12": ("q11", "m12")}
_OUTPUTS = {
    (0, 0): {"m1": 1, "m2": 1, "q8": 1, "m13": 1, "m15": 1},
    (0, 1): {"m3": 1, "m7": 1, "q12": 1},
    (0, 2): {"m5": 1, "q12": 1, "m15": 1},
    (1, 0): {"m2": 1, "q9": 1, "m14": 1},
    (1, 1): {"m4": 1, "q9": 1, "m10": 1},
    (1, 2): {"m5": 1, "m6": 1, "q11": 1, "m13": -1, "m14": 1},
}


def _left_operands(a):
    (a00, a01, a02), (a10, a11, a12) = a
    s1, s6 = a00 - a10, a02 - a12
    s7, s8 = a00 + a01, s1 + a01
    s9, s10, s11 = s8 - a11, a11 + a12, a11 - s6
    s12, s13, s14, s15 = s11 - a01, a10 + a02, a10 + a12, a00 + a02
    ops = (s1, a10, a01, a11, a02, s6, s7, s8, s9, s10, s11, s12, s13, s14, s15)
    return {r: v.astype(jnp.bfloat16) for r, v in zip(_PRODUCTS, ops)}


def _right_operand(r, block):
    pos = [block(*pq) for pq, sign in _RIGHT[r].items() if sign > 0]
    neg = [block(*pq) for pq, sign in _RIGHT[r].items() if sign < 0]
    total = functools.reduce(lambda u, v: u + v, pos) if pos else -neg.pop()
    return functools.reduce(lambda u, v: u - v, neg, total)


class _BlockProduct:
    def __init__(self, emit):
        self.emit = emit
        self.ready, self.partial = {}, {}
        self.missing = {iq: dict(terms) for iq, terms in _OUTPUTS.items()}

    def add(self, r, product):
        fresh = ["m%d" % r]
        self.ready[fresh[0]] = product
        for name, (u, v) in _SHARED.items():
            if name not in self.ready and u in self.ready and v in self.ready:
                self.ready[name] = self.ready[u] + self.ready[v]
                fresh.append(name)
        complete = [iq for iq, terms in self.missing.items() if all(name in self.ready for name in terms)]
        for iq in complete:
            self._fold(iq, fresh)
            self.emit(*iq, self.partial[iq][1])
            del self.missing[iq]
        for name in fresh:
            for iq in self.missing:
                self._fold(iq, [name])

    def _fold(self, iq, names):
        for name in names:
            if name not in self.missing[iq]:
                continue
            sign, value = self.missing[iq].pop(name), self.ready[name]
            if iq in self.partial:
                have, total = self.partial[iq]
                if have == sign:
                    value = total + value
                else:
                    sign, value = 1, (total - value if have > 0 else value - total)
            self.partial[iq] = (sign, value)


def _pack(v):
    return pltpu.bitcast(v.astype(jnp.bfloat16), jnp.uint32)


def _unpack(v):
    return pltpu.bitcast(v, jnp.bfloat16)


def _kernel(x_hbm, dw_ref, w1_hbm, w2_hbm, g_ref, b_ref, o_hbm, h_hbm,
            xbuf, hbuf, wc, lhs0, acc, xsem, osem, hsem, *, cfg):
    TM, NCACHE, NS, NX, U = (cfg[k] for k in ("TM", "NCACHE", "NS", "NX", "U"))
    R1, R2, AHEAD, SLACK = (cfg[k] for k in ("R1", "R2", "AHEAD", "SLACK"))
    F, C = w2_hbm.shape
    CB, FB = C // 3, F // 3
    T = x_hbm.shape[0] // TM
    NSPILL = T - NCACHE - NS
    NW = pl.cdiv(F, TM)
    f32, bf16 = jnp.float32, jnp.bfloat16

    def place(t):
        span = T - NS
        before = jnp.minimum(t * NCACHE // span, NCACHE)
        ring = jnp.minimum((t + 1) * NCACHE // span, NCACHE) == before
        s = t - before
        return ring, s, jnp.where(ring, s % NS, NS + before)

    def nowhere(placed):
        return (jnp.logical_and(placed[0], False), *placed[1:])

    def x_load(t):
        return pltpu.make_async_copy(x_hbm.at[pl.ds(t * TM, TM)], xbuf.at[t % NX, pl.ds(0, TM)], xsem.at[t % NX])

    def o_store(t):
        return pltpu.make_async_copy(xbuf.at[t % NX, pl.ds(0, TM)], o_hbm.at[pl.ds(t * TM, TM)], osem.at[t % NX])

    def h_store(s):
        return pltpu.make_async_copy(hbuf.at[s % NS], h_hbm.at[s], hsem.at[s % NS])

    def h_load(s):
        return pltpu.make_async_copy(h_hbm.at[s], hbuf.at[s % NS], hsem.at[s % NS])

    def w2_load(k):
        n, slot = min(TM, F - k * TM), (T + k) % NX
        return pltpu.make_async_copy(w2_hbm.at[pl.ds(k * TM, n)], xbuf.at[slot, pl.ds(0, n)], xsem.at[slot])

    def w2_tile(r0, c0):
        return xbuf[(T + r0 // TM) % NX, r0 % TM:r0 % TM + CB, c0:c0 + CB]

    def h_block(slot, r0, n, p):
        return jnp.concatenate(
            [hbuf[slot, p * (FB // CB) + k, r0:r0 + n, :].astype(f32) for k in range(FB // CB)], axis=1)

    def layernorm(t, r0, n):
        y = xbuf[t % NX, r0:r0 + n, :].astype(f32) * dw
        d = y - jnp.sum(y, axis=-1, keepdims=True) * (1.0 / C)
        v = jnp.sum(d * d, axis=-1, keepdims=True) + C * _LN_EPS
        return d * jnp.exp2(-0.5 * jnp.log2(v))

    def operands1(rows):
        return _left_operands([[u[:, p * CB:(p + 1) * CB] for p in range(3)] for u in rows])

    staging = NS + NCACHE - 1
    w1_loads = [pltpu.make_async_copy(w1_hbm.at[:, pl.ds(j * CB, CB)], hbuf.at[staging, j, pl.ds(0, C)], hsem.at[0])
                for j in range(F // CB)]
    x_load(0).start()
    for load in w1_loads:
        load.start()
    for t in range(1, U + 1):
        x_load(t).start()
    acc[...] = jnp.zeros_like(acc)
    dw = dw_ref[...].astype(f32)
    x_load(0).wait()
    for sub in range(AHEAD):
        for r, v in operands1([layernorm(0, (2 * sub + i) * R1, R1) for i in range(2)]).items():
            lhs0[sub, r - 1] = v
    for load in w1_loads:
        load.wait()
    for r in _PRODUCTS:
        wc[r - 1] = _pack((_BETA * math.sqrt(C)) * _right_operand(r, lambda p, q: h_block(staging, p * CB, CB, q)))

    def sweep1(it, carry):
        t0 = it * U
        done, tiles = carry
        for ring, s, _ in tiles:
            @pl.when(jnp.logical_and(ring, s >= NS))
            def _():
                h_store(s - NS).wait()
        for u in range(1, U):
            x_load(t0 + u).wait()

        @pl.when(t0 + U < T)
        def _():
            x_load(t0 + U).wait()

        @pl.when(t0 + U == T)
        def _():
            w2_load(0).wait()

        def start_copies():
            for ring, s, _ in done:
                @pl.when(jnp.logical_and(ring, s < NSPILL))
                def _():
                    h_store(s).start()
            for t in [t0 + U + 1 + u for u in range(U)]:
                @pl.when(t < T)
                def _():
                    x_load(t).start()
            for k in range(NW):
                @pl.when(it == (T + k - U - 1) // U)
                def _():
                    w2_load(k).start()

        per_tile = TM // (2 * R1)
        nsub = U * per_tile
        sumsq = {}
        operands = {sub: {r: lhs0[sub, r - 1] for r in _PRODUCTS} for sub in range(AHEAD)}

        def emit(sub, c, i, q, w):
            h = w * jnp.tanh(w * (w * w + _KAPPA)) + w
            r0, j = (sub % per_tile * 2 + i) * R1, q * (FB // CB) + c
            hbuf[tiles[sub // per_tile][2], j, r0:r0 + R1, :] = h.astype(bf16)
            sq = jnp.sum((h * h).reshape(R1 // 8, 8, CB), axis=0)
            sumsq[j] = sumsq[j] + sq if j in sumsq else sq

        def stream(c):
            gates = cfg["GATES"]
            n_rows = 2 * R1 // len(gates)
            for sub in range(nsub):
                block_product = _BlockProduct(functools.partial(emit, sub, c))
                pieces = []
                for n, r in enumerate(cfg["ORDER1"][c]):
                    m = jnp.dot(operands[sub][r], _unpack(wc[r - 1, :, c * CB:(c + 1) * CB]),
                                preferred_element_type=f32)
                    block_product.add(r, m)
                    for k, gate in enumerate(gates if c == 0 else ()):
                        last = sub == nsub - 1
                        if n == (0 if last else gate):
                            if not last:
                                xbuf[(t0 + U + 1) % NX, TM:TM + 8, 0:CB] = m[0:8].astype(xbuf.dtype)
                            later = sub + AHEAD
                            r0 = later % per_tile * 2 * R1 + k % 2 * R1 + k // 2 * n_rows
                            pieces.append(layernorm(t0 + later // per_tile, r0, n_rows))
                    yield
                if c == 0:
                    operands[sub + AHEAD] = operands1([jnp.concatenate(pieces[i::2], axis=0) for i in range(2)])

        streams = [stream(c) for c in range(FB // CB)]
        for n in range(15 * nsub + max(cfg["LAG"])):
            for steps, lag in zip(streams, cfg["LAG"]):
                if 0 <= n - lag < 15 * nsub:
                    next(steps)
            if n == 2:
                start_copies()
        for steps in streams:
            next(steps, None)
        for j, v in sumsq.items():
            acc[:, j * CB:(j + 1) * CB] += v
        for sub in range(AHEAD):
            for r, v in operands[nsub + sub].items():
                lhs0[sub, r - 1] = v
        return tiles, [place(t0 + U + u) for u in range(U)]

    first = [place(jnp.int32(u)) for u in range(U)]
    jax.lax.fori_loop(0, T // U, sweep1, ([nowhere(p) for p in first], first))

    gx = jnp.sqrt(jnp.sum(acc[...], axis=0, keepdims=True) * _HSCALE ** 2 + _GRN_EPS)
    nx = gx / (jnp.sum(gx, axis=-1, keepdims=True) * (1.0 / F) + _GRN_EPS)
    scale = (g_ref[...].astype(f32).reshape(1, F) * nx + 1.0) * _HSCALE
    for k in range(1, NW):
        w2_load(k).wait()
    for k in range(FB // CB):
        rows = [p * FB + k * CB for p in range(3)]
        col = [jnp.transpose(jnp.broadcast_to(scale[:, r0:r0 + CB], (CB, CB))) for r0 in rows]
        scaled = [[w2_tile(rows[p], q * CB).astype(f32) * col[p] for q in range(3)] for p in range(3)]
        for r in _PRODUCTS:
            wc[r - 1, :, k * CB:(k + 1) * CB] = _pack(_right_operand(r, lambda p, q: scaled[p][q]))
    w2 = jnp.concatenate([jnp.concatenate([w2_tile(r0, c0) for c0 in range(0, C, CB)], axis=1)
                          for r0 in range(0, F, CB)], axis=0)
    b = jnp.broadcast_to(b_ref[...].astype(f32).reshape(1, F), (16, F)).astype(bf16)
    bias = jnp.dot(b, w2, preferred_element_type=f32)[0:1, :]
    for k in reversed(range(NW)):
        x_load(T - NX + k).start()

    def sweep2(step, carry):
        t = T - 1 - step
        (done_ring, done_s, _), (ring, s, slot) = carry

        @pl.when(t + SLACK < T)
        def _():
            o_store(t + SLACK).wait()

        @pl.when(jnp.logical_and(ring, s < NSPILL))
        def _():
            h_load(s).wait()

        @pl.when(t < T - NX + NW)
        def _():
            x_load(t).wait()

        @pl.when(step > 0)
        def _():
            o_store(t + 1).start()

        @pl.when(jnp.logical_and(t + SLACK < T, t + SLACK >= NX))
        def _():
            x_load(t + SLACK - NX).start()

        for r0 in range(0, TM, 2 * R2):
            if r0 == 2 * R2:
                @pl.when(jnp.logical_and(done_ring, done_s >= NS))
                def _():
                    h_load(done_s - NS).start()

            def emit(i, q, y):
                rows, cols = slice(r0 + i * R2, r0 + (i + 1) * R2), slice(q * CB, (q + 1) * CB)
                xbuf[t % NX, rows, cols] = (
                    y + bias[:, cols] + xbuf[t % NX, rows, cols].astype(f32)).astype(xbuf.dtype)

            ops = _left_operands([[h_block(slot, r0 + i * R2, R2, p) for p in range(3)] for i in range(2)])
            block_product = _BlockProduct(emit)
            for r in cfg["ORDER2"]:
                w = jnp.concatenate(
                    [_unpack(wc[r - 1, :, k * CB:(k + 1) * CB]) for k in range(FB // CB)], axis=0)
                block_product.add(r, jnp.dot(ops[r], w, preferred_element_type=f32))
        return (ring, s, slot), place(jnp.maximum(t - 1, 0))

    last = place(jnp.int32(T - 1))
    jax.lax.fori_loop(0, T, sweep2, (nowhere(last), last))
    o_store(0).start()
    for t in range(SLACK):
        o_store(t).wait()


_DEFAULT_CFG = dict(
    TM=1152,
    NCACHE=31, NS=4,
    NX=6, SLACK=2,
    U=2,
    R1=48, R2=64,
    ORDER1=((7, 8, 9, 11, 10, 2, 4, 13, 14, 6, 12, 3, 5, 15, 1), (7, 8, 11, 10, 9, 2, 4, 13, 14, 6, 3, 12, 5, 15, 1),
            (7, 8, 9, 2, 10, 4, 6, 14, 13, 11, 12, 3, 5, 15, 1), (7, 2, 9, 8, 10, 4, 6, 14, 13, 5, 11, 12, 3, 15, 1)),
    LAG=(0, 4, 8, 11), GATES=(3, 3, 4, 6, 10, 14), AHEAD=2,
    ORDER2=(5, 2, 1, 8, 9, 7, 4, 3, 6, 11, 10, 13, 12, 15, 14),
)


def _run(x, dw, w1, w2, grn_g, grn_b, cfg):
    B, H, W, C = x.shape
    F = w1.shape[1]
    N, TM = H * W, cfg["TM"]
    assert B == 1 and dw.shape == (1, 1, C) and C == 3 * 128 and F == 4 * C and x.dtype == jnp.bfloat16
    assert N % (TM * cfg["U"]) == 0 and cfg["NX"] > 2 * cfg["U"] and cfg["NS"] >= 2 * cfg["U"] and cfg["SLACK"] >= 2
    n_spilled = N // TM - cfg["NCACHE"] - cfg["NS"]
    hbm, vmem = pl.BlockSpec(memory_space=pl.ANY), pl.BlockSpec(memory_space=pltpu.VMEM)
    out, _ = pl.pallas_call(
        functools.partial(_kernel, cfg=cfg),
        in_specs=[hbm, vmem, hbm, hbm, vmem, vmem],
        out_specs=[hbm, hbm],
        out_shape=[
            jax.ShapeDtypeStruct((N, C), x.dtype),
            jax.ShapeDtypeStruct((n_spilled, F // 128, TM, 128), jnp.bfloat16),
        ],
        scratch_shapes=[
            pltpu.VMEM((cfg["NX"], TM + 16, C), x.dtype),
            pltpu.VMEM((cfg["NS"] + cfg["NCACHE"], F // 128, TM, 128), jnp.bfloat16),
            pltpu.VMEM((15, C // 6, F // 3), jnp.uint32),
            pltpu.VMEM((cfg["AHEAD"], 15, cfg["R1"], C // 3), jnp.bfloat16),
            pltpu.VMEM((8, F), jnp.float32),
            pltpu.SemaphoreType.DMA((cfg["NX"],)),
            pltpu.SemaphoreType.DMA((cfg["NX"],)),
            pltpu.SemaphoreType.DMA((cfg["NS"],)),
        ],
        compiler_params=pltpu.CompilerParams(vmem_limit_bytes=int(127.9 * 2 ** 20), disable_bounds_checks=True),
    )(x.reshape(N, C), dw.reshape(1, C), w1.astype(jnp.bfloat16), w2.astype(jnp.bfloat16), grn_g, grn_b)
    return out.reshape(B, H, W, C)


@jax.jit
def pallas_standalone__modern_conv_block_slak__vision_kernel(
    x: jax.Array,
    dw: jax.Array,
    w1: jax.Array,
    w2: jax.Array,
    grn_g: jax.Array,
    grn_b: jax.Array,
):
    return _run(x, dw, w1, w2, grn_g, grn_b, _DEFAULT_CFG)
```

```python
import functools
import math

import jax
import jax.numpy as jnp
import jax.experimental.pallas as pl
import jax.experimental.pallas.tpu as pltpu

_LN_EPS = 1e-5
_GRN_EPS = 1e-6
_C0 = math.sqrt(2.0 / math.pi)
_BETA = (0.044715 * _C0) ** (1.0 / 3.0)
_KAPPA = _C0 / _BETA
_HSCALE = 1.0 / (2.0 * _BETA)

_PRODUCTS = tuple(range(1, 16))
_RIGHT = {
    1: {(0, 0): 1, (0, 2): -1, (1, 0): -1},
    2: {(0, 0): 1, (0, 1): -1, (2, 0): -1},
    3: {(1, 1): 1, (0, 1): -1, (1, 2): -1},
    4: {(1, 1): 1, (1, 0): -1, (2, 1): -1},
    5: {(2, 2): 1, (0, 2): -1, (2, 1): -1},
    6: {(1, 2): 1, (2, 0): 1, (2, 2): -1},
    7: {(0, 1): 1},
    8: {(1, 0): 1, (0, 1): -1},
    9: {(1, 0): -1},
    10: {(2, 1): 1},
    11: {(1, 2): 1, (2, 1): -1},
    12: {(1, 2): -1},
    13: {(2, 0): 1, (0, 2): -1},
    14: {(2, 0): 1},
    15: {(0, 2): 1},
}
_SHARED = {"q8": ("m7", "m8"), "q9": ("q8", "m9"), "q11": ("m10", "m11"), "q12": ("q11", "m12")}
_OUTPUTS = {
    (0, 0): {"m1": 1, "m2": 1, "q8": 1, "m13": 1, "m15": 1},
    (0, 1): {"m3": 1, "m7": 1, "q12": 1},
    (0, 2): {"m5": 1, "q12": 1, "m15": 1},
    (1, 0): {"m2": 1, "q9": 1, "m14": 1},
    (1, 1): {"m4": 1, "q9": 1, "m10": 1},
    (1, 2): {"m5": 1, "m6": 1, "q11": 1, "m13": -1, "m14": 1},
}


def _left_operands(a):
    (a00, a01, a02), (a10, a11, a12) = a
    s1, s6 = a00 - a10, a02 - a12
    s7, s8 = a00 + a01, s1 + a01
    s9, s10, s11 = s8 - a11, a11 + a12, a11 - s6
    s12, s13, s14, s15 = s11 - a01, a10 + a02, a10 + a12, a00 + a02
    ops = (s1, a10, a01, a11, a02, s6, s7, s8, s9, s10, s11, s12, s13, s14, s15)
    return {r: v.astype(jnp.bfloat16) for r, v in zip(_PRODUCTS, ops)}


def _right_operand(r, block):
    pos = [block(*pq) for pq, sign in _RIGHT[r].items() if sign > 0]
    neg = [block(*pq) for pq, sign in _RIGHT[r].items() if sign < 0]
    total = functools.reduce(lambda u, v: u + v, pos) if pos else -neg.pop()
    return functools.reduce(lambda u, v: u - v, neg, total)


class _BlockProduct:
    def __init__(self, emit):
        self.emit = emit
        self.ready, self.partial = {}, {}
        self.missing = {iq: dict(terms) for iq, terms in _OUTPUTS.items()}

    def add(self, r, product):
        fresh = ["m%d" % r]
        self.ready[fresh[0]] = product
        for name, (u, v) in _SHARED.items():
            if name not in self.ready and u in self.ready and v in self.ready:
                self.ready[name] = self.ready[u] + self.ready[v]
                fresh.append(name)
        complete = [iq for iq, terms in self.missing.items() if all(name in self.ready for name in terms)]
        for iq in complete:
            self._fold(iq, fresh)
            self.emit(*iq, self.partial[iq][1])
            del self.missing[iq]
        for name in fresh:
            for iq in self.missing:
                self._fold(iq, [name])

    def _fold(self, iq, names):
        for name in names:
            if name not in self.missing[iq]:
                continue
            sign, value = self.missing[iq].pop(name), self.ready[name]
            if iq in self.partial:
                have, total = self.partial[iq]
                if have == sign:
                    value = total + value
                else:
                    sign, value = 1, (total - value if have > 0 else value - total)
            self.partial[iq] = (sign, value)


def _pack(v):
    return pltpu.bitcast(v.astype(jnp.bfloat16), jnp.uint32)


def _unpack(v):
    return pltpu.bitcast(v, jnp.bfloat16)


def _kernel(x_hbm, dw_ref, w1_hbm, w2_hbm, g_ref, b_ref, o_hbm, h_hbm,
            xbuf, hbuf, wc, lhs0, acc, xsem, osem, hsem, *, cfg):
    TM, NCACHE, NS, NX, U = (cfg[k] for k in ("TM", "NCACHE", "NS", "NX", "U"))
    R1, R2, AHEAD, SLACK = (cfg[k] for k in ("R1", "R2", "AHEAD", "SLACK"))
    F, C = w2_hbm.shape
    CB, FB = C // 3, F // 3
    T = x_hbm.shape[0] // TM
    NSPILL = T - NCACHE - NS
    NW = pl.cdiv(F, TM)
    f32, bf16 = jnp.float32, jnp.bfloat16

    def place(t):
        span = T - NS
        before = jnp.minimum(t * NCACHE // span, NCACHE)
        ring = jnp.minimum((t + 1) * NCACHE // span, NCACHE) == before
        s = t - before
        return ring, s, jnp.where(ring, s % NS, NS + before)

    def nowhere(placed):
        return (jnp.logical_and(placed[0], False), *placed[1:])

    def x_load(t):
        return pltpu.make_async_copy(x_hbm.at[pl.ds(t * TM, TM)], xbuf.at[t % NX, pl.ds(0, TM)], xsem.at[t % NX])

    def o_store(t):
        return pltpu.make_async_copy(xbuf.at[t % NX, pl.ds(0, TM)], o_hbm.at[pl.ds(t * TM, TM)], osem.at[t % NX])

    def h_store(s):
        return pltpu.make_async_copy(hbuf.at[s % NS], h_hbm.at[s], hsem.at[s % NS])

    def h_load(s, r0):
        rows = pl.ds(r0, 2 * R2)
        return pltpu.make_async_copy(h_hbm.at[s, :, rows], hbuf.at[s % NS, :, rows], hsem.at[s % NS])

    def w2_load(k):
        n, slot = min(TM, F - k * TM), (T + k) % NX
        return pltpu.make_async_copy(w2_hbm.at[pl.ds(k * TM, n)], xbuf.at[slot, pl.ds(0, n)], xsem.at[slot])

    def w2_tile(r0, c0):
        return xbuf[(T + r0 // TM) % NX, r0 % TM:r0 % TM + CB, c0:c0 + CB]

    def h_block(slot, r0, n, p):
        return jnp.concatenate(
            [hbuf[slot, p * (FB // CB) + k, r0:r0 + n, :].astype(f32) for k in range(FB // CB)], axis=1)

    def layernorm(t, r0, n):
        y = xbuf[t % NX, r0:r0 + n, :].astype(f32) * dw
        d = y - jnp.sum(y, axis=-1, keepdims=True) * (1.0 / C)
        v = jnp.sum(d * d, axis=-1, keepdims=True) + C * _LN_EPS
        return d * jnp.exp2(-0.5 * jnp.log2(v))

    def operands1(rows):
        return _left_operands([[u[:, p * CB:(p + 1) * CB] for p in range(3)] for u in rows])

    staging = NS + NCACHE - 1
    w1_loads = [pltpu.make_async_copy(w1_hbm.at[:, pl.ds(j * CB, CB)], hbuf.at[staging, j, pl.ds(0, C)], hsem.at[0])
                for j in range(F // CB)]
    x_load(0).start()
    for load in w1_loads:
        load.start()
    for t in range(1, U + 1):
        x_load(t).start()
    acc[...] = jnp.zeros_like(acc)
    dw = dw_ref[...].astype(f32)
    x_load(0).wait()
    for sub in range(AHEAD):
        for r, v in operands1([layernorm(0, (2 * sub + i) * R1, R1) for i in range(2)]).items():
            lhs0[sub, r - 1] = v
    for load in w1_loads:
        load.wait()
    for r in _PRODUCTS:
        wc[r - 1] = _pack((_BETA * math.sqrt(C)) * _right_operand(r, lambda p, q: h_block(staging, p * CB, CB, q)))

    def sweep1(it, carry):
        t0 = it * U
        done, tiles = carry
        for ring, s, _ in tiles:
            @pl.when(jnp.logical_and(ring, s >= NS))
            def _():
                h_store(s - NS).wait()
        for u in range(1, U):
            x_load(t0 + u).wait()

        @pl.when(t0 + U < T)
        def _():
            x_load(t0 + U).wait()

        @pl.when(t0 + U == T)
        def _():
            w2_load(0).wait()

        def start_copies():
            for ring, s, _ in done:
                @pl.when(jnp.logical_and(ring, s < NSPILL))
                def _():
                    h_store(s).start()
            for t in [t0 + U + 1 + u for u in range(U)]:
                @pl.when(t < T)
                def _():
                    x_load(t).start()
            for k in range(NW):
                @pl.when(it == (T + k - U - 1) // U)
                def _():
                    w2_load(k).start()

        per_tile = TM // (2 * R1)
        nsub = U * per_tile
        sumsq = {}
        operands = {sub: {r: lhs0[sub, r - 1] for r in _PRODUCTS} for sub in range(AHEAD)}

        def emit(sub, c, i, q, w):
            h = w * jnp.tanh(w * (w * w + _KAPPA)) + w
            r0, j = (sub % per_tile * 2 + i) * R1, q * (FB // CB) + c
            hbuf[tiles[sub // per_tile][2], j, r0:r0 + R1, :] = h.astype(bf16)
            sq = jnp.sum((h * h).reshape(R1 // 8, 8, CB), axis=0)
            sumsq[j] = sumsq[j] + sq if j in sumsq else sq

        def stream(c):
            gates = cfg["GATES"]
            n_rows = 2 * R1 // len(gates)
            for sub in range(nsub):
                block_product = _BlockProduct(functools.partial(emit, sub, c))
                pieces = []
                for n, r in enumerate(cfg["ORDER1"][c]):
                    m = jnp.dot(operands[sub][r], _unpack(wc[r - 1, :, c * CB:(c + 1) * CB]),
                                preferred_element_type=f32)
                    block_product.add(r, m)
                    for k, gate in enumerate(gates if c == 0 else ()):
                        last = sub == nsub - 1
                        if n == (0 if last else gate):
                            if not last:
                                xbuf[(t0 + U + 1) % NX, TM:TM + 8, 0:CB] = m[0:8].astype(xbuf.dtype)
                            later = sub + AHEAD
                            r0 = later % per_tile * 2 * R1 + k % 2 * R1 + k // 2 * n_rows
                            pieces.append(layernorm(t0 + later // per_tile, r0, n_rows))
                    yield
                if c == 0:
                    operands[sub + AHEAD] = operands1([jnp.concatenate(pieces[i::2], axis=0) for i in range(2)])

        streams = [stream(c) for c in range(FB // CB)]
        for n in range(15 * nsub + max(cfg["LAG"])):
            for steps, lag in zip(streams, cfg["LAG"]):
                if 0 <= n - lag < 15 * nsub:
                    next(steps)
            if n == 2:
                start_copies()
        for steps in streams:
            next(steps, None)
        for j, v in sumsq.items():
            acc[:, j * CB:(j + 1) * CB] += v
        for sub in range(AHEAD):
            for r, v in operands[nsub + sub].items():
                lhs0[sub, r - 1] = v
        return tiles, [place(t0 + U + u) for u in range(U)]

    first = [place(jnp.int32(u)) for u in range(U)]
    jax.lax.fori_loop(0, T // U, sweep1, ([nowhere(p) for p in first], first))

    gx = jnp.sqrt(jnp.sum(acc[...], axis=0, keepdims=True) * _HSCALE ** 2 + _GRN_EPS)
    nx = gx / (jnp.sum(gx, axis=-1, keepdims=True) * (1.0 / F) + _GRN_EPS)
    scale = (g_ref[...].astype(f32).reshape(1, F) * nx + 1.0) * _HSCALE
    for k in range(1, NW):
        w2_load(k).wait()
    for k in range(FB // CB):
        rows = [p * FB + k * CB for p in range(3)]
        col = [jnp.transpose(jnp.broadcast_to(scale[:, r0:r0 + CB], (CB, CB))) for r0 in rows]
        scaled = [[w2_tile(rows[p], q * CB).astype(f32) * col[p] for q in range(3)] for p in range(3)]
        for r in _PRODUCTS:
            wc[r - 1, :, k * CB:(k + 1) * CB] = _pack(_right_operand(r, lambda p, q: scaled[p][q]))
    w2 = jnp.concatenate([jnp.concatenate([w2_tile(r0, c0) for c0 in range(0, C, CB)], axis=1)
                          for r0 in range(0, F, CB)], axis=0)
    b = jnp.broadcast_to(b_ref[...].astype(f32).reshape(1, F), (16, F)).astype(bf16)
    bias = jnp.dot(b, w2, preferred_element_type=f32)[0:1, :]
    for k in reversed(range(NW)):
        x_load(T - NX + k).start()

    def sweep2(step, carry):
        t = T - 1 - step
        (done_ring, done_s, _), (ring, s, slot) = carry

        @pl.when(t + SLACK < T)
        def _():
            o_store(t + SLACK).wait()

        @pl.when(jnp.logical_and(ring, s < NSPILL))
        def _():
            for r0 in range(0, TM, 2 * R2):
                h_load(s, r0).wait()

        @pl.when(t < T - NX + NW)
        def _():
            x_load(t).wait()

        @pl.when(step > 0)
        def _():
            o_store(t + 1).start()

        @pl.when(jnp.logical_and(t + SLACK < T, t + SLACK >= NX))
        def _():
            x_load(t + SLACK - NX).start()

        for r0 in range(0, TM, 2 * R2):
            if r0 == 2 * R2:
                @pl.when(jnp.logical_and(done_ring, done_s >= NS))
                def _():
                    h_load(done_s - NS, TM - 2 * R2).start()
            if r0 > 0:
                @pl.when(jnp.logical_and(ring, s >= NS))
                def _():
                    h_load(s - NS, r0 - 2 * R2).start()

            def emit(i, q, y):
                rows, cols = slice(r0 + i * R2, r0 + (i + 1) * R2), slice(q * CB, (q + 1) * CB)
                xbuf[t % NX, rows, cols] = (
                    y + bias[:, cols] + xbuf[t % NX, rows, cols].astype(f32)).astype(xbuf.dtype)

            ops = _left_operands([[h_block(slot, r0 + i * R2, R2, p) for p in range(3)] for i in range(2)])
            block_product = _BlockProduct(emit)
            for r in cfg["ORDER2"]:
                w = jnp.concatenate(
                    [_unpack(wc[r - 1, :, k * CB:(k + 1) * CB]) for k in range(FB // CB)], axis=0)
                block_product.add(r, jnp.dot(ops[r], w, preferred_element_type=f32))
        return (ring, s, slot), place(jnp.maximum(t - 1, 0))

    last = place(jnp.int32(T - 1))
    jax.lax.fori_loop(0, T, sweep2, (nowhere(last), last))
    o_store(0).start()
    for t in range(SLACK):
        o_store(t).wait()


_DEFAULT_CFG = dict(
    TM=1152,
    NCACHE=31, NS=4,
    NX=6, SLACK=2,
    U=2,
    R1=48, R2=64,
    ORDER1=((7, 8, 9, 11, 2, 4, 10, 5, 14, 6, 12, 3, 15, 13, 1), (11, 2, 8, 7, 9, 10, 4, 13, 14, 6, 3, 12, 5, 15, 1),
            (8, 7, 9, 2, 10, 4, 6, 14, 13, 11, 12, 3, 5, 15, 1), (9, 2, 8, 7, 10, 4, 6, 14, 13, 5, 11, 12, 3, 15, 1)),
    LAG=(0, 4, 8, 11), GATES=(3, 3, 4, 6, 10, 14), AHEAD=2,
    ORDER2=(5, 1, 2, 8, 7, 9, 4, 3, 15, 6, 11, 10, 14, 12, 13),
)


def _run(x, dw, w1, w2, grn_g, grn_b, cfg):
    B, H, W, C = x.shape
    F = w1.shape[1]
    N, TM = H * W, cfg["TM"]
    assert B == 1 and dw.shape == (1, 1, C) and C == 3 * 128 and F == 4 * C and x.dtype == jnp.bfloat16
    assert N % (TM * cfg["U"]) == 0 and cfg["NX"] > 2 * cfg["U"] and cfg["NS"] >= 2 * cfg["U"] and cfg["SLACK"] >= 2
    n_spilled = N // TM - cfg["NCACHE"] - cfg["NS"]
    hbm, vmem = pl.BlockSpec(memory_space=pl.ANY), pl.BlockSpec(memory_space=pltpu.VMEM)
    out, _ = pl.pallas_call(
        functools.partial(_kernel, cfg=cfg),
        in_specs=[hbm, vmem, hbm, hbm, vmem, vmem],
        out_specs=[hbm, hbm],
        out_shape=[
            jax.ShapeDtypeStruct((N, C), x.dtype),
            jax.ShapeDtypeStruct((n_spilled, F // 128, TM, 128), jnp.bfloat16),
        ],
        scratch_shapes=[
            pltpu.VMEM((cfg["NX"], TM + 16, C), x.dtype),
            pltpu.VMEM((cfg["NS"] + cfg["NCACHE"], F // 128, TM, 128), jnp.bfloat16),
            pltpu.VMEM((15, C // 6, F // 3), jnp.uint32),
            pltpu.VMEM((cfg["AHEAD"], 15, cfg["R1"], C // 3), jnp.bfloat16),
            pltpu.VMEM((8, F), jnp.float32),
            pltpu.SemaphoreType.DMA((cfg["NX"],)),
            pltpu.SemaphoreType.DMA((cfg["NX"],)),
            pltpu.SemaphoreType.DMA((cfg["NS"],)),
        ],
        compiler_params=pltpu.CompilerParams(vmem_limit_bytes=int(127.9 * 2 ** 20), disable_bounds_checks=True),
    )(x.reshape(N, C), dw.reshape(1, C), w1.astype(jnp.bfloat16), w2.astype(jnp.bfloat16), grn_g, grn_b)
    return out.reshape(B, H, W, C)


@jax.jit
def pallas_standalone__modern_conv_block_slak__vision_kernel(
    x: jax.Array,
    dw: jax.Array,
    w1: jax.Array,
    w2: jax.Array,
    grn_g: jax.Array,
    grn_b: jax.Array,
):
    return _run(x, dw, w1, w2, grn_g, grn_b, _DEFAULT_CFG)
```
